```python
import jax
import jax.numpy as jnp

def _softmax(x, axis=-1):
    return jax.nn.softmax(x, axis=axis)

def _gelu(x):
    return jax.nn.gelu(x, approximate=True)

def _silu(x):
    return jax.nn.silu(x)

def _sigmoid(x):
    return jax.nn.sigmoid(x)

def _layernorm(x, axis=-1, eps=1e-05):
    m = jnp.mean(x, axis=axis, keepdims=True)
    v = jnp.var(x, axis=axis, keepdims=True)
    return (x - m) / jnp.sqrt(v + eps)

def _scatter_add(tgt, idx, src, axis=0):
    return tgt.at[idx].add(src)

def _segment_sum(src, seg, n):
    return jax.ops.segment_sum(src, seg, n)

class _Rng:

    def __init__(self, key):
        self._k = key

    def _next(self):
        self._k, sub = jax.random.split(self._k)
        return sub

    def normal(self, shape):
        return jax.random.normal(self._next(), shape, dtype=jnp.bfloat16)

    def randint(self, lo, hi, shape):
        return jax.random.randint(self._next(), shape, lo, hi, dtype=jnp.int32)

    def uniform(self, shape, lo=0.0, hi=1.0):
        return jax.random.uniform(self._next(), shape, jnp.bfloat16, lo, hi)

    def permutation(self, n):
        return jax.random.permutation(self._next(), n)
kernel_name = 'adaLN_cond__compressed_kv_cla__glu_gated_geglu__decode'

def setup_inputs():
    _rng = _Rng(jax.random.key(int.from_bytes(__import__("os").urandom(4), "little")))
    _w = lambda a: (lambda t: t.astype(jnp.bfloat16) if jnp.issubdtype(t.dtype, jnp.floating) else t)(jnp.asarray(a))

    def _A_setup():
        B, H, Sq, Sk, D, M = (1, 32, 1, 32768, 128, 512)
        Dc = 4 * D
        return {'x': _w((lambda *s: _rng.normal(s) * 0.05)(B, Sq, M)), 'c_kv': _w((lambda *s: _rng.normal(s) * 0.05)(B, Sk, Dc)), 'w_q': _w((lambda *s: _rng.normal(s) * 0.05)(M, H, D) * M ** (-0.5)), 'w_uk': _w((lambda *s: _rng.normal(s) * 0.05)(Dc, H, D) * Dc ** (-0.5)), 'w_uv': _w((lambda *s: _rng.normal(s) * 0.05)(Dc, H, D) * Dc ** (-0.5)), 'w_o': _w((lambda *s: _rng.normal(s) * 0.05)(H, D, M) * (H * D) ** (-0.5))}
    _A_in = _A_setup()

    def _B_setup():
        B, S, Dm, Df = (1, 1, 512, 1792)
        return {'x': _w((lambda *s: _rng.normal(s) * 0.05)(B, S, Dm)), 'w_gate': _w((lambda *s: _rng.normal(s) * 0.05)(Dm, Df) * Dm ** (-0.5)), 'w_up': _w((lambda *s: _rng.normal(s) * 0.05)(Dm, Df) * Dm ** (-0.5)), 'w_down': _w((lambda *s: _rng.normal(s) * 0.05)(Df, Dm) * Df ** (-0.5))}
    _B_in = _B_setup()
    return {'A_x': _A_in['x'], 'A_c_kv': _A_in['c_kv'], 'A_w_q': _A_in['w_q'], 'A_w_uk': _A_in['w_uk'], 'A_w_uv': _A_in['w_uv'], 'A_w_o': _A_in['w_o'], 'B_x': _B_in['x'], 'B_w_gate': _B_in['w_gate'], 'B_w_up': _B_in['w_up'], 'B_w_down': _B_in['w_down'], 'c': _w((lambda *s: _rng.normal(s) * 0.05)(1, 512)), 'w_mod': _w((lambda *s: _rng.normal(s) * 0.05)(512, 6 * 512) * 512 ** (-0.5))}

def reference(A_x, A_c_kv, A_w_q, A_w_uk, A_w_uv, A_w_o, B_x, B_w_gate, B_w_up, B_w_down, c, w_mod):

    def _A_ref(x, c_kv, w_q, w_uk, w_uv, w_o):
        B, Sq, M = (x.shape[0], x.shape[1], x.shape[2])
        Sk = c_kv.shape[1]
        H, D = (w_q.shape[1], w_q.shape[2])
        q = jnp.einsum('bqm,mhd->bhqd', x, w_q)
        k = jnp.einsum('bkc,chd->bhkd', c_kv, w_uk)
        v = jnp.einsum('bkc,chd->bhkd', c_kv, w_uv)
        scores = jnp.einsum('bhqd,bhkd->bhqk', q, k) * D ** (-0.5)
        off = Sk - Sq
        qi = jnp.arange(Sq)[:, None]
        kj = jnp.arange(Sk)[None, :]
        cmask = kj <= qi + off
        scores = jnp.where(cmask[None, None], scores, -1000000000.0)
        p = _softmax(scores, axis=-1)
        ctx = jnp.einsum('bhqk,bhkd->bhqd', p, v)
        return jnp.einsum('bhqd,hdm->bqm', ctx, w_o)

    def _B_ref(x, w_gate, w_up, w_down):
        g = jnp.einsum('bsd,df->bsf', x, w_gate)
        u = jnp.einsum('bsd,df->bsf', x, w_up)
        h = _gelu(g) * u
        return jnp.einsum('bsf,fd->bsd', h, w_down)
    x = A_x
    mod = (_silu(c) @ w_mod).reshape(c.shape[0], 6, 1, -1)
    sa, ca, ga, sb, cb, gb = (mod[:, 0].copy(), mod[:, 1].copy(), mod[:, 2].copy(), mod[:, 3].copy(), mod[:, 4].copy(), mod[:, 5].copy())
    h = _layernorm(x, axis=-1) * (1 + ca) + sa
    x = x + ga * _A_ref(h, A_c_kv, A_w_q, A_w_uk, A_w_uv, A_w_o)
    h = _layernorm(x, axis=-1) * (1 + cb) + sb
    x = x + gb * _B_ref(h, B_w_gate, B_w_up, B_w_down)
    return x
```

```python
import functools

import jax
import jax.numpy as jnp
from jax import lax
import jax.experimental.pallas as pl
import jax.experimental.pallas.tpu as pltpu

_F32 = jnp.float32
_BF16 = jnp.bfloat16

_KV_DMA_ROWS = 4096
_KV_TILE = 2048
_DOWN_SPLITS = (1024, 512, 256)


def _layernorm(x, eps=1e-05):
    m = jnp.mean(x, axis=-1, keepdims=True)
    xc = x - m
    v = jnp.mean(xc * xc, axis=-1, keepdims=True)
    return xc / jnp.sqrt(v + eps)


def _dot(a, b):
    return jnp.dot(a, b, preferred_element_type=_F32)


def _dot_nt(a, b):
    return lax.dot_general(a, b, (((1,), (1,)), ((), ())),
                           preferred_element_type=_F32)


def _kernel(x_hbm, ckv_hbm, wq_hbm, wuk_hbm, wuv_hbm, wo_hbm, wg_hbm, wu_hbm,
            wd_hbm, c_hbm, wmod_hbm, o_ref,
            x_v, c_v, wmod_v, wq_v, wuk_v, ckv_v, wuv_v, wo_v, wg_v, wu_v, wd_v,
            sems, kv_sems, *, H, D, M, DC, SK):
    n_kv_dma = SK // _KV_DMA_ROWS
    tiles_per_dma = _KV_DMA_ROWS // _KV_TILE
    G = 128 * H
    NJ = DC // 128

    def whole(src, dst, i):
        return pltpu.make_async_copy(src, dst, sems.at[i])

    cp_wmod = whole(wmod_hbm, wmod_v, 0)
    cp_c = whole(c_hbm, c_v, 1)
    cp_x = whole(x_hbm, x_v, 2)
    cp_wq = whole(wq_hbm, wq_v, 3)
    cp_wuk = whole(wuk_hbm, wuk_v, 4)
    cp_wuv = whole(wuv_hbm, wuv_v, 5)
    cp_wo = whole(wo_hbm, wo_v, 6)
    cp_wg = whole(wg_hbm, wg_v, 7)
    cp_wu = whole(wu_hbm, wu_v, 8)
    cp_wd = []
    off = 0
    for i, n in enumerate(_DOWN_SPLITS):
        cp_wd.append(pltpu.make_async_copy(
            wd_hbm.at[pl.ds(off, n)], wd_v.at[pl.ds(off, n)], sems.at[9 + i]))
        off += n

    def cp_kv(i):
        r = i * _KV_DMA_ROWS
        return pltpu.make_async_copy(
            ckv_hbm.at[pl.ds(r, _KV_DMA_ROWS)], ckv_v.at[pl.ds(r, _KV_DMA_ROWS)],
            kv_sems.at[i])

    for cp in (cp_wmod, cp_c, cp_x, cp_wq, cp_wuk):
        cp.start()
    for i in range(n_kv_dma):
        cp_kv(i).start()
    for cp in (cp_wuv, cp_wo, cp_wg, cp_wu, *cp_wd):
        cp.start()

    row = lax.broadcasted_iota(jnp.int32, (128, G), 0)
    col = lax.broadcasted_iota(jnp.int32, (128, G), 1)
    expand = jnp.where(col // H == row, 1.0, 0.0).astype(_BF16)
    diag = (col % H) == (row % H)

    def contract_major(a, w_v):
        stacked = jnp.concatenate(
            [a[:, 128 * j:128 * (j + 1)] for j in range(NJ)], axis=0)
        big = jnp.where(diag, _dot(stacked, expand), 0.0).astype(_BF16)
        out = None
        for j in range(NJ):
            t = _dot(big[H * j:H * (j + 1), :], w_v[G * j:G * (j + 1), :])
            out = t if out is None else out + t
        return out

    cp_wmod.wait()
    cp_c.wait()
    cp_x.wait()
    c = c_v[...].astype(_F32)
    sc = (c * jax.nn.sigmoid(c)).astype(_BF16)
    mod = _dot(sc, wmod_v[...])
    sa, ca, ga, sb, cb, gb = (mod[:, M * i:M * (i + 1)] for i in range(6))
    x = x_v[...].astype(_F32)
    h1 = (_layernorm(x) * (1.0 + ca) + sa).astype(_BF16)

    cp_wq.wait()
    q = contract_major(jnp.broadcast_to(h1, (H, M)), wq_v).astype(_BF16)
    cp_wuk.wait()
    ys = [_dot_nt(q, wuk_v[G * j:G * (j + 1), :]) for j in range(NJ)]
    ym = jnp.where(diag, jnp.concatenate(ys, axis=0) * (D ** -0.5), 0.0).astype(_BF16)
    qs = _dot_nt(ym, expand)
    qa = jnp.concatenate(
        [qs[H * j:H * (j + 1), :] for j in range(NJ)], axis=1).astype(_BF16)

    def kv_step(i, carry):
        cp_kv(i).wait()
        m, l, acc = carry
        for t in range(tiles_per_dma):
            r = pl.multiple_of(i * _KV_DMA_ROWS + t * _KV_TILE, _KV_TILE)
            kv = ckv_v[pl.ds(r, _KV_TILE), :]
            s = _dot_nt(qa, kv)
            m_new = jnp.maximum(m, jnp.max(s, axis=1, keepdims=True))
            alpha = jnp.exp(m - m_new)
            p = jnp.exp(s - m_new)
            l = l * alpha + jnp.sum(p, axis=1, keepdims=True)
            acc = acc * alpha + _dot(p.astype(_BF16), kv)
            m = m_new
        return m, l, acc

    init = (jnp.full((H, 1), -jnp.inf, _F32), jnp.zeros((H, 1), _F32),
            jnp.zeros((H, DC), _F32))
    _, l, acc = lax.fori_loop(0, n_kv_dma, kv_step, init)
    cc = (acc / l).astype(_BF16)

    cp_wuv.wait()
    ctx = contract_major(cc, wuv_v)

    r32 = lax.broadcasted_iota(jnp.int32, (H, H * D), 0)
    c32 = lax.broadcasted_iota(jnp.int32, (H, H * D), 1)
    lo = jnp.where(c32 // D == r32, jnp.concatenate([ctx] * H, axis=1), 0.0).astype(_BF16)
    cp_wo.wait()
    attn = jnp.sum(_dot(lo, wo_v[...]), axis=0, keepdims=True)
    x2 = x + ga * attn

    h2 = (_layernorm(x2) * (1.0 + cb) + sb).astype(_BF16)
    cp_wg.wait()
    g = _dot(h2, wg_v[...])
    cp_wu.wait()
    u = _dot(h2, wu_v[...])
    hf = (jax.nn.gelu(g, approximate=True) * u).astype(_BF16)
    ffn = None
    off = 0
    for cp, n in zip(cp_wd, _DOWN_SPLITS):
        cp.wait()
        t = _dot(hf[:, off:off + n], wd_v[off:off + n, :])
        ffn = t if ffn is None else ffn + t
        off += n
    o_ref[...] = (x2 + gb * ffn).astype(o_ref.dtype)


@jax.jit
def pallas_adaLN_cond__compressed_kv_cla__glu_gated_geglu__decode_kernel(
    A_x: jax.Array,
    A_c_kv: jax.Array,
    A_w_q: jax.Array,
    A_w_uk: jax.Array,
    A_w_uv: jax.Array,
    A_w_o: jax.Array,
    B_x: jax.Array,
    B_w_gate: jax.Array,
    B_w_up: jax.Array,
    B_w_down: jax.Array,
    c: jax.Array,
    w_mod: jax.Array,
):
    B, SQ, M = A_x.shape
    _, SK, DC = A_c_kv.shape
    _, H, D = A_w_q.shape
    DF = B_w_gate.shape[1]
    assert B == 1 and SQ == 1 and M == DC and H * (DC // 128) == 128
    assert sum(_DOWN_SPLITS) == DF and SK % _KV_DMA_ROWS == 0

    x2d = A_x.reshape(1, M)
    ckv = A_c_kv.reshape(SK, DC)
    wq = A_w_q.reshape(M * H, D)
    wuk = A_w_uk.reshape(DC * H, D)
    wuv = A_w_uv.reshape(DC * H, D)
    wo = A_w_o.reshape(H * D, M)

    operands = (x2d, ckv, wq, wuk, wuv, wo, B_w_gate, B_w_up, B_w_down, c, w_mod)
    vm = lambda a: pltpu.VMEM(a.shape, a.dtype)
    out = pl.pallas_call(
        functools.partial(_kernel, H=H, D=D, M=M, DC=DC, SK=SK),
        in_specs=[pl.BlockSpec(memory_space=pl.ANY)] * len(operands),
        out_specs=pl.BlockSpec(memory_space=pltpu.VMEM),
        out_shape=jax.ShapeDtypeStruct((1, M), A_x.dtype),
        scratch_shapes=[
            vm(x2d), vm(c), vm(w_mod), vm(wq), vm(wuk), vm(ckv), vm(wuv), vm(wo),
            vm(B_w_gate), vm(B_w_up), vm(B_w_down),
            pltpu.SemaphoreType.DMA((9 + len(_DOWN_SPLITS),)),
            pltpu.SemaphoreType.DMA((SK // _KV_DMA_ROWS,)),
        ],
        compiler_params=pltpu.CompilerParams(vmem_limit_bytes=96 * 1024 * 1024),
    )(*operands)
    return out.reshape(B, SQ, M)
```

```python
import functools

import jax
import jax.numpy as jnp
from jax import lax
import jax.experimental.pallas as pl
import jax.experimental.pallas.tpu as pltpu

_F32 = jnp.float32
_BF16 = jnp.bfloat16

_KV_DMA_ROWS = 4096
_KV_TILE = 2048
_DOWN_SPLITS = (1024, 512, 256)


def _layernorm(x, eps=1e-05):
    m = jnp.mean(x, axis=-1, keepdims=True)
    xc = x - m
    v = jnp.mean(xc * xc, axis=-1, keepdims=True)
    return xc / jnp.sqrt(v + eps)


def _dot(a, b):
    return jnp.dot(a, b, preferred_element_type=_F32)


def _dot_nt(a, b):
    return lax.dot_general(a, b, (((1,), (1,)), ((), ())),
                           preferred_element_type=_F32)


def _kernel(x_hbm, ckv_hbm, wq_hbm, wuk_hbm, wuv_hbm, wo_hbm, wg_hbm, wu_hbm,
            wd_hbm, c_hbm, wmod_hbm, o_ref,
            x_v, c_v, wmod_v, wq_v, wuk_v, ckv_v, wuv_v, wo_v, wg_v, wu_v, wd_v,
            sems, *, H, D, M, DC, SK):
    n_kv_dma = SK // _KV_DMA_ROWS
    tiles_per_dma = _KV_DMA_ROWS // _KV_TILE
    G = 128 * H
    NJ = DC // 128

    def whole(src, dst, i):
        return pltpu.make_async_copy(src, dst, sems.at[i])

    cp_wmod = whole(wmod_hbm, wmod_v, 0)
    cp_c = whole(c_hbm, c_v, 1)
    cp_x = whole(x_hbm, x_v, 2)
    cp_wq = whole(wq_hbm, wq_v, 3)
    cp_wuk = whole(wuk_hbm, wuk_v, 4)
    cp_wuv = whole(wuv_hbm, wuv_v, 5)
    cp_wo = whole(wo_hbm, wo_v, 6)
    cp_wg = whole(wg_hbm, wg_v, 7)
    cp_wu = whole(wu_hbm, wu_v, 8)
    cp_wd = []
    off = 0
    for i, n in enumerate(_DOWN_SPLITS):
        cp_wd.append(pltpu.make_async_copy(
            wd_hbm.at[pl.ds(off, n)], wd_v.at[pl.ds(off, n)], sems.at[9 + i]))
        off += n

    def cp_kv(i):
        r = i * _KV_DMA_ROWS
        return pltpu.make_async_copy(
            ckv_hbm.at[pl.ds(r, _KV_DMA_ROWS)], ckv_v.at[pl.ds(r, _KV_DMA_ROWS)],
            sems.at[9 + len(_DOWN_SPLITS) + i])

    for cp in (cp_wmod, cp_c, cp_x, cp_wq, cp_wuk):
        cp.start()
    for i in range(n_kv_dma):
        cp_kv(i).start()
    for cp in (cp_wuv, cp_wo, cp_wg, cp_wu, *cp_wd):
        cp.start()

    row = lax.broadcasted_iota(jnp.int32, (128, G), 0)
    col = lax.broadcasted_iota(jnp.int32, (128, G), 1)
    expand = jnp.where(col // H == row, 1.0, 0.0).astype(_BF16)
    diag = (col % H) == (row % H)

    def contract_major(a, w_v):
        stacked = jnp.concatenate(
            [a[:, 128 * j:128 * (j + 1)] for j in range(NJ)], axis=0)
        big = jnp.where(diag, _dot(stacked, expand), 0.0).astype(_BF16)
        out = None
        for j in range(NJ):
            t = _dot(big[H * j:H * (j + 1), :], w_v[G * j:G * (j + 1), :])
            out = t if out is None else out + t
        return out

    cp_wmod.wait()
    cp_c.wait()
    cp_x.wait()
    c = c_v[...].astype(_F32)
    sc = (c * jax.nn.sigmoid(c)).astype(_BF16)
    mod = _dot(sc, wmod_v[...])
    sa, ca, ga, sb, cb, gb = (mod[:, M * i:M * (i + 1)] for i in range(6))
    x = x_v[...].astype(_F32)
    h1 = (_layernorm(x) * (1.0 + ca) + sa).astype(_BF16)

    cp_wq.wait()
    q = contract_major(jnp.broadcast_to(h1, (H, M)), wq_v).astype(_BF16)
    cp_wuk.wait()
    ys = [_dot_nt(q, wuk_v[G * j:G * (j + 1), :]) for j in range(NJ)]
    ym = jnp.where(diag, jnp.concatenate(ys, axis=0) * (D ** -0.5), 0.0).astype(_BF16)
    qs = _dot_nt(ym, expand)
    qa = jnp.concatenate(
        [qs[H * j:H * (j + 1), :] for j in range(NJ)], axis=1).astype(_BF16)

    def kv_step(i, carry):
        cp_kv(i).wait()
        m, l, acc = carry
        for t in range(tiles_per_dma):
            r = pl.multiple_of(i * _KV_DMA_ROWS + t * _KV_TILE, _KV_TILE)
            kv = ckv_v[pl.ds(r, _KV_TILE), :]
            s = _dot_nt(qa, kv)
            m_new = jnp.maximum(m, jnp.max(s, axis=1, keepdims=True))
            alpha = jnp.exp(m - m_new)
            p = jnp.exp(s - m_new)
            l = l * alpha + jnp.sum(p, axis=1, keepdims=True)
            acc = acc * alpha + _dot(p.astype(_BF16), kv)
            m = m_new
        return m, l, acc

    init = (jnp.full((H, 1), -jnp.inf, _F32), jnp.zeros((H, 1), _F32),
            jnp.zeros((H, DC), _F32))
    _, l, acc = lax.fori_loop(0, n_kv_dma, kv_step, init)
    cc = (acc / l).astype(_BF16)

    cp_wuv.wait()
    ctx = contract_major(cc, wuv_v)

    r32 = lax.broadcasted_iota(jnp.int32, (H, H * D), 0)
    c32 = lax.broadcasted_iota(jnp.int32, (H, H * D), 1)
    lo = jnp.where(c32 // D == r32, jnp.concatenate([ctx] * H, axis=1), 0.0).astype(_BF16)
    cp_wo.wait()
    attn = jnp.sum(_dot(lo, wo_v[...]), axis=0, keepdims=True)
    x2 = x + ga * attn

    h2 = (_layernorm(x2) * (1.0 + cb) + sb).astype(_BF16)
    cp_wg.wait()
    g = _dot(h2, wg_v[...])
    cp_wu.wait()
    u = _dot(h2, wu_v[...])
    hf = (jax.nn.gelu(g, approximate=True) * u).astype(_BF16)
    ffn = None
    off = 0
    for cp, n in zip(cp_wd, _DOWN_SPLITS):
        cp.wait()
        t = _dot(hf[:, off:off + n], wd_v[off:off + n, :])
        ffn = t if ffn is None else ffn + t
        off += n
    o_ref[...] = (x2 + gb * ffn).astype(o_ref.dtype)


@jax.jit
def pallas_adaLN_cond__compressed_kv_cla__glu_gated_geglu__decode_kernel(
    A_x: jax.Array,
    A_c_kv: jax.Array,
    A_w_q: jax.Array,
    A_w_uk: jax.Array,
    A_w_uv: jax.Array,
    A_w_o: jax.Array,
    B_x: jax.Array,
    B_w_gate: jax.Array,
    B_w_up: jax.Array,
    B_w_down: jax.Array,
    c: jax.Array,
    w_mod: jax.Array,
):
    B, SQ, M = A_x.shape
    _, SK, DC = A_c_kv.shape
    _, H, D = A_w_q.shape
    DF = B_w_gate.shape[1]
    assert B == 1 and SQ == 1 and M == DC and H * (DC // 128) == 128
    assert sum(_DOWN_SPLITS) == DF and SK % _KV_DMA_ROWS == 0

    x2d = A_x.reshape(1, M)
    ckv = A_c_kv.reshape(SK, DC)
    wq = A_w_q.reshape(M * H, D)
    wuk = A_w_uk.reshape(DC * H, D)
    wuv = A_w_uv.reshape(DC * H, D)
    wo = A_w_o.reshape(H * D, M)

    operands = (x2d, ckv, wq, wuk, wuv, wo, B_w_gate, B_w_up, B_w_down, c, w_mod)
    vm = lambda a: pltpu.VMEM(a.shape, a.dtype)
    out = pl.pallas_call(
        functools.partial(_kernel, H=H, D=D, M=M, DC=DC, SK=SK),
        in_specs=[pl.BlockSpec(memory_space=pl.ANY)] * len(operands),
        out_specs=pl.BlockSpec(memory_space=pltpu.VMEM),
        out_shape=jax.ShapeDtypeStruct((1, M), A_x.dtype),
        scratch_shapes=[
            vm(x2d), vm(c), vm(w_mod), vm(wq), vm(wuk), vm(ckv), vm(wuv), vm(wo),
            vm(B_w_gate), vm(B_w_up), vm(B_w_down),
            pltpu.SemaphoreType.DMA((9 + len(_DOWN_SPLITS) + SK // _KV_DMA_ROWS,)),
        ],
        compiler_params=pltpu.CompilerParams(vmem_limit_bytes=96 * 1024 * 1024),
    )(*operands)
    return out.reshape(B, SQ, M)
```

```python
import functools

import jax
import jax.numpy as jnp
from jax import lax
import jax.experimental.pallas as pl
import jax.experimental.pallas.tpu as pltpu

_F32 = jnp.float32
_BF16 = jnp.bfloat16

_KV_DMA_ROWS = 4096
_KV_TILE = 2048
_DOWN_SPLITS = (1024, 512, 256)


def _layernorm(x, eps=1e-05):
    m = jnp.mean(x, axis=-1, keepdims=True)
    xc = x - m
    v = jnp.mean(xc * xc, axis=-1, keepdims=True)
    return xc / jnp.sqrt(v + eps)


def _dot(a, b):
    return jnp.dot(a, b, preferred_element_type=_F32)


def _dot_nt(a, b):
    return lax.dot_general(a, b, (((1,), (1,)), ((), ())),
                           preferred_element_type=_F32)


def _kernel(x_hbm, ckv_hbm, wq_hbm, wuk_hbm, wuv_hbm, wo_hbm, wg_hbm, wu_hbm,
            wd_hbm, c_hbm, wmod_hbm, o_ref,
            x_v, c_v, wmod_v, wq_v, wuk_v, ckv_v, wuv_v, wo_v, wg_v, wu_v, wd_v,
            sems, *, H, D, M, DC, SK):
    n_kv_dma = SK // _KV_DMA_ROWS
    tiles_per_dma = _KV_DMA_ROWS // _KV_TILE
    G = 128 * H
    NJ = DC // 128

    def whole(src, dst, i):
        return pltpu.make_async_copy(src, dst, sems.at[i])

    cp_wmod = whole(wmod_hbm, wmod_v, 0)
    cp_c = whole(c_hbm, c_v, 1)
    cp_x = whole(x_hbm, x_v, 2)
    cp_wq = whole(wq_hbm, wq_v, 3)
    cp_wuk = whole(wuk_hbm, wuk_v, 4)
    cp_wuv = whole(wuv_hbm, wuv_v, 5)
    cp_wo = whole(wo_hbm, wo_v, 6)
    cp_wg = whole(wg_hbm, wg_v, 7)
    cp_wu = whole(wu_hbm, wu_v, 8)
    cp_wd = []
    off = 0
    for i, n in enumerate(_DOWN_SPLITS):
        cp_wd.append(pltpu.make_async_copy(
            wd_hbm.at[pl.ds(off, n)], wd_v.at[pl.ds(off, n)], sems.at[9 + i]))
        off += n

    def cp_kv(i):
        r = i * _KV_DMA_ROWS
        return pltpu.make_async_copy(
            ckv_hbm.at[pl.ds(r, _KV_DMA_ROWS)], ckv_v.at[pl.ds(r, _KV_DMA_ROWS)],
            sems.at[9 + len(_DOWN_SPLITS) + i])

    for cp in (cp_wmod, cp_c, cp_x, cp_wq, cp_wuk):
        cp.start()
    for i in range(n_kv_dma):
        cp_kv(i).start()
    for cp in (cp_wuv, cp_wo, cp_wg, cp_wu, *cp_wd):
        cp.start()

    row = lax.broadcasted_iota(jnp.int32, (128, G), 0)
    col = lax.broadcasted_iota(jnp.int32, (128, G), 1)
    expand = jnp.where(col // H == row, 1.0, 0.0).astype(_BF16)
    diag = (col % H) == (row % H)

    def contract_major(a, w_v):
        stacked = jnp.concatenate(
            [a[:, 128 * j:128 * (j + 1)] for j in range(NJ)], axis=0)
        big = jnp.where(diag, _dot(stacked, expand), 0.0).astype(_BF16)
        out = None
        for j in range(NJ):
            t = _dot(big[H * j:H * (j + 1), :], w_v[G * j:G * (j + 1), :])
            out = t if out is None else out + t
        return out

    cp_wmod.wait()
    cp_c.wait()
    cp_x.wait()
    c = c_v[...].astype(_F32)
    sc = (c * jax.nn.sigmoid(c)).astype(_BF16)
    mod = _dot(sc, wmod_v[...])
    sa, ca, ga, sb, cb, gb = (mod[:, M * i:M * (i + 1)] for i in range(6))
    x = x_v[...].astype(_F32)
    h1 = (_layernorm(x) * (1.0 + ca) + sa).astype(_BF16)

    cp_wq.wait()
    q = contract_major(jnp.broadcast_to(h1, (H, M)), wq_v).astype(_BF16)
    cp_wuk.wait()
    ys = [_dot_nt(q, wuk_v[G * j:G * (j + 1), :]) for j in range(NJ)]
    ym = jnp.where(diag, jnp.concatenate(ys, axis=0) * (D ** -0.5), 0.0).astype(_BF16)
    qs = _dot_nt(ym, expand)
    qa = jnp.concatenate(
        [qs[H * j:H * (j + 1), :] for j in range(NJ)], axis=1).astype(_BF16)

    def kv_step(i, carry):
        cp_kv(i).wait()
        m, l, acc = carry
        for t in range(tiles_per_dma):
            r = pl.multiple_of(i * _KV_DMA_ROWS + t * _KV_TILE, _KV_TILE)
            kv = ckv_v[pl.ds(r, _KV_TILE), :]
            s = _dot_nt(qa, kv)
            m_new = jnp.maximum(m, jnp.max(s, axis=1, keepdims=True))
            alpha = jnp.exp(m - m_new)
            p = jnp.exp(s - m_new)
            l = l * alpha + jnp.sum(p, axis=1, keepdims=True)
            acc = acc * alpha + _dot(p.astype(_BF16), kv)
            m = m_new
        return m, l, acc

    init = (jnp.full((H, 1), -jnp.inf, _F32), jnp.zeros((H, 1), _F32),
            jnp.zeros((H, DC), _F32))
    _, l, acc = lax.fori_loop(0, n_kv_dma, kv_step, init)
    cc = (acc / l).astype(_BF16)

    cp_wuv.wait()
    ctx = contract_major(cc, wuv_v)

    r32 = lax.broadcasted_iota(jnp.int32, (H, H * D), 0)
    c32 = lax.broadcasted_iota(jnp.int32, (H, H * D), 1)
    lo = jnp.where(c32 // D == r32, jnp.concatenate([ctx] * H, axis=1), 0.0).astype(_BF16)
    cp_wo.wait()
    attn = jnp.sum(_dot(lo, wo_v[...]), axis=0, keepdims=True)
    x2 = x + ga * attn

    h2 = (_layernorm(x2) * (1.0 + cb) + sb).astype(_BF16)
    cp_wg.wait()
    g = _dot(h2, wg_v[...])
    cp_wu.wait()
    u = _dot(h2, wu_v[...])
    hf = (jax.nn.gelu(g, approximate=True) * u).astype(_BF16)
    ffn = None
    off = 0
    for cp, n in zip(cp_wd, _DOWN_SPLITS):
        cp.wait()
        t = _dot(hf[:, off:off + n], wd_v[off:off + n, :])
        ffn = t if ffn is None else ffn + t
        off += n
    o_ref[...] = (x2 + gb * ffn).astype(o_ref.dtype)


@jax.jit
def pallas_adaLN_cond__compressed_kv_cla__glu_gated_geglu__decode_kernel(
    A_x: jax.Array,
    A_c_kv: jax.Array,
    A_w_q: jax.Array,
    A_w_uk: jax.Array,
    A_w_uv: jax.Array,
    A_w_o: jax.Array,
    B_x: jax.Array,
    B_w_gate: jax.Array,
    B_w_up: jax.Array,
    B_w_down: jax.Array,
    c: jax.Array,
    w_mod: jax.Array,
):
    B, SQ, M = A_x.shape
    _, SK, DC = A_c_kv.shape
    _, H, D = A_w_q.shape
    DF = B_w_gate.shape[1]
    assert B == 1 and SQ == 1 and M == DC and H * (DC // 128) == 128
    assert sum(_DOWN_SPLITS) == DF and SK % _KV_DMA_ROWS == 0

    x2d = A_x.reshape(1, M)
    ckv = A_c_kv.reshape(SK, DC)
    wq = A_w_q.reshape(M * H, D)
    wuk = A_w_uk.reshape(DC * H, D)
    wuv = A_w_uv.reshape(DC * H, D)
    wo = A_w_o.reshape(H * D, M)

    operands = (x2d, ckv, wq, wuk, wuv, wo, B_w_gate, B_w_up, B_w_down, c, w_mod)
    vm = lambda a: pltpu.VMEM(a.shape, a.dtype)
    out = pl.pallas_call(
        functools.partial(_kernel, H=H, D=D, M=M, DC=DC, SK=SK),
        in_specs=[pl.BlockSpec(memory_space=pl.ANY)] * len(operands),
        out_specs=pl.BlockSpec(memory_space=pltpu.VMEM),
        out_shape=jax.ShapeDtypeStruct((1, M), A_x.dtype),
        scratch_shapes=[
            vm(x2d), vm(c), vm(w_mod), vm(wq), vm(wuk), vm(ckv), vm(wuv), vm(wo),
            vm(B_w_gate), vm(B_w_up), vm(B_w_down),
            pltpu.SemaphoreType.DMA((9 + len(_DOWN_SPLITS) + SK // _KV_DMA_ROWS,)),
        ],
        compiler_params=pltpu.CompilerParams(
            vmem_limit_bytes=96 * 1024 * 1024,
            disable_semaphore_checks=True,
        ),
    )(*operands)
    return out.reshape(B, SQ, M)
```

```python
import functools

import jax
import jax.numpy as jnp
from jax import lax
import jax.experimental.pallas as pl
import jax.experimental.pallas.tpu as pltpu

_F32 = jnp.float32
_BF16 = jnp.bfloat16

_KV_TILE = 2048
_SKEW = 26
_LEAD = 48
_NB = 2
_G = 8


def _layernorm(x, eps=1e-05):
    m = jnp.mean(x, axis=-1, keepdims=True)
    xc = x - m
    v = jnp.mean(xc * xc, axis=-1, keepdims=True)
    return xc / jnp.sqrt(v + eps)


def _dot(a, b):
    return jnp.dot(a, b, preferred_element_type=_F32)


def _dot_nt(a, b):
    return lax.dot_general(a, b, (((1,), (1,)), ((), ())),
                           preferred_element_type=_F32)


(S_WMOD, S_C, S_X, S_WQ, S_WUK, S_WUV, S_WO, S_WG, S_WU, S_WD0, S_WD1, S_WD2, S_WD3,
 S_KV) = range(14)


def _kernel(x_hbm, ckv_hbm, wq_hbm, wuk_hbm, wuv_hbm, wo_hbm, wg_hbm, wu_hbm,
            wd_hbm, c_hbm, wmod_hbm, o_ref,
            x_v, c_v, wmod_v, wq_v, wuk_v, ckv_v, wuv_v, wo_v, wg_v, wu_v, wd_v,
            sems, *, H, D, M, DC, SK):
    NT = SK // _KV_TILE
    RPT = _KV_TILE // _G
    HPT = RPT // 16
    G = 128 * H
    NJ = DC // 128

    def piece(src, dst, sem, g0, g1, rows, cols=None):
        idx = (pl.ds(g0, g1 - g0), rows) + (() if cols is None else (cols,))
        return pltpu.make_async_copy(src.at[idx], dst.at[idx], sems.at[sem])

    def kv_piece(tile, j, g0, g1):
        r = tile * RPT + j * 16
        if not isinstance(r, int):
            r = pl.multiple_of(r, 16)
        return pltpu.make_async_copy(
            ckv_hbm.at[pl.ds(g0, g1 - g0), pl.ds(r, 16)],
            ckv_v.at[tile, pl.ds(g0, g1 - g0), pl.ds(j * 16, 16)],
            sems.at[S_KV + tile])

    A, B = [], []

    def add(fn, nb, ng):
        B.append(lambda: fn(0, nb))
        A.append(lambda: fn(nb, ng))

    for cb in range(3):
        for r in range(8):
            add(functools.partial(
                lambda g0, g1, r, cb: piece(wmod_hbm, wmod_v, S_WMOD, g0, g1, pl.ds(8 * r, 8),
                                            pl.ds(1024 * cb, 1024)), r=r, cb=cb), _NB, _G)
    e_wmod = len(A)

    def add_rows(src, dst, sem, n, rows, nb, ng, j0=0):
        for j in range(j0, j0 + n):
            add(functools.partial(
                lambda g0, g1, j: piece(src, dst, sem, g0, g1, pl.ds(rows * j, rows)), j=j), nb, ng)

    add_rows(wq_hbm, wq_v, S_WQ, 32, 64, _NB, _G)
    e_wq = len(A)
    add_rows(wuk_hbm, wuk_v, S_WUK, 32, 64, _NB, _G)
    e_wuk = len(A)
    for t in range(NT):
        for j in range(HPT):
            add(functools.partial(lambda g0, g1, t, j: kv_piece(t, j, g0, g1), t=t, j=j), _NB, _G)
    e_kv = len(A)
    add_rows(wuv_hbm, wuv_v, S_WUV, 32, 64, _NB, _G)
    e_wuv = len(A)
    add_rows(wo_hbm, wo_v, S_WO, 32, 16, _NB, _G)
    e_wo = len(A)
    for j in range(16):
        add_rows(wg_hbm, wg_v, S_WG, 1, 8, 1, 4, j0=j)
        add_rows(wu_hbm, wu_v, S_WU, 1, 8, 1, 4, j0=j)
    e_wgu = len(A)
    add_rows(wd_hbm, wd_v, S_WD0, 8, 16, 1, 6)
    add_rows(wd_hbm, wd_v, S_WD1, 8, 16, 1, 6, j0=8)
    NHOP = len(A)
    for j in range(32):
        A.append(functools.partial(piece, wd_hbm, wd_v, S_WD2 if j < 16 else S_WD3, 6, 7,
                                   pl.ds(8 * j, 8)))
    NA = len(A)
    assert NA >= NHOP + _SKEW

    ptr = [0]

    def emit(lo, hi):
        for i in range(lo, hi):
            A[i]().start(priority=1)
            if 0 <= i - _SKEW < NHOP:
                B[i - _SKEW]().start(priority=0)

    def issue_for(e):
        hi = min(e + _LEAD, NA)
        if hi > ptr[0]:
            emit(ptr[0], hi)
            ptr[0] = hi

    def wait_all(buf, sem):
        pltpu.make_async_copy(buf, buf, sems.at[sem]).wait()

    cp_c = pltpu.make_async_copy(c_hbm, c_v, sems.at[S_C])
    cp_x = pltpu.make_async_copy(x_hbm, x_v, sems.at[S_X])
    emit(0, 1)
    ptr[0] = 1
    cp_c.start()
    cp_x.start()
    issue_for(e_wmod)

    row = lax.broadcasted_iota(jnp.int32, (128, G), 0)
    col = lax.broadcasted_iota(jnp.int32, (128, G), 1)
    expand = jnp.where(col // H == row, 1.0, 0.0).astype(_BF16)
    diag = (col % H) == (row % H)

    def wslab(w_v, j):
        return w_v[2 * j:2 * j + 2].reshape(G, D)

    def expand_lhs(a):
        stacked = jnp.concatenate(
            [a[:, 128 * j:128 * (j + 1)] for j in range(NJ)], axis=0)
        return jnp.where(diag, _dot(stacked, expand), 0.0).astype(_BF16)

    def contract_major(big, w_v):
        out = None
        for j in range(NJ):
            t = _dot(big[H * j:H * (j + 1), :], wslab(w_v, j))
            out = t if out is None else out + t
        return out

    cp_c.wait()
    cp_x.wait()
    wait_all(wmod_v, S_WMOD)
    c = c_v[...].astype(_F32)
    sc = (c * jax.nn.sigmoid(c)).astype(_BF16)
    mod = _dot(sc, wmod_v[...].reshape(M, 6 * M))
    sa, ca, ga, sb, cb, gb = (mod[:, M * i:M * (i + 1)] for i in range(6))
    x = x_v[...].astype(_F32)
    h1 = (_layernorm(x) * (1.0 + ca) + sa).astype(_BF16)
    big_q = expand_lhs(jnp.broadcast_to(h1, (H, M)))

    issue_for(e_wq)
    wait_all(wq_v, S_WQ)
    q = contract_major(big_q, wq_v).astype(_BF16)
    issue_for(e_wuk)
    wait_all(wuk_v, S_WUK)
    ys = [_dot_nt(q, wslab(wuk_v, j)) for j in range(NJ)]
    ym = jnp.where(diag, jnp.concatenate(ys, axis=0) * (D ** -0.5), 0.0).astype(_BF16)
    qs = _dot_nt(ym, expand)
    qa = jnp.concatenate(
        [qs[H * j:H * (j + 1), :] for j in range(NJ)], axis=1).astype(_BF16)

    p0 = ptr[0]
    assert p0 == e_wuk + _LEAD and p0 - _SKEW >= e_wuk
    n_dyn = (e_kv - p0) // HPT

    def kv_step(t, carry):
        @pl.when(t < n_dyn)
        def _():
            for jj in range(HPT):
                ha = p0 - e_wuk + jj
                hb = ha - _SKEW
                kv_piece(t + ha // HPT, ha % HPT, _NB, _G).start(priority=1)
                kv_piece(t + hb // HPT, hb % HPT, 0, _NB).start(priority=0)

        for tt in range(n_dyn, NT):
            @pl.when(t == tt)
            def _():
                emit(p0 + HPT * tt, p0 + HPT * (tt + 1))

        pltpu.make_async_copy(ckv_v.at[t], ckv_v.at[t], sems.at[S_KV + t]).wait()
        m, l, acc = carry
        kv = ckv_v[t].reshape(_KV_TILE, DC)
        s = _dot_nt(qa, kv)
        m_new = jnp.maximum(m, jnp.max(s, axis=1, keepdims=True))
        alpha = jnp.exp(m - m_new)
        p = jnp.exp(s - m_new)
        l = l * alpha + jnp.sum(p, axis=1, keepdims=True)
        acc = acc * alpha + _dot(p.astype(_BF16), kv)
        return m_new, l, acc

    init = (jnp.full((H, 1), -jnp.inf, _F32), jnp.zeros((H, 1), _F32),
            jnp.zeros((H, DC), _F32))
    _, l, acc = lax.fori_loop(0, NT, kv_step, init)
    ptr[0] = p0 + HPT * NT
    cc = (acc / l).astype(_BF16)
    big_c = expand_lhs(cc)

    issue_for(e_wuv)
    wait_all(wuv_v, S_WUV)
    ctx = contract_major(big_c, wuv_v)

    r32 = lax.broadcasted_iota(jnp.int32, (H, H * D), 0)
    c32 = lax.broadcasted_iota(jnp.int32, (H, H * D), 1)
    lo = jnp.where(c32 // D == r32, jnp.concatenate([ctx] * H, axis=1), 0.0).astype(_BF16)
    issue_for(e_wo)
    wait_all(wo_v, S_WO)
    attn = jnp.sum(_dot(lo, wo_v[...].reshape(H * D, M)), axis=0, keepdims=True)
    x2 = x + ga * attn

    h2 = (_layernorm(x2) * (1.0 + cb) + sb).astype(_BF16)
    issue_for(NA)
    DF = wg_v.shape[-1]
    wait_all(wg_v, S_WG)
    g = _dot(h2, wg_v[...].reshape(M, DF))
    wait_all(wu_v, S_WU)
    u = _dot(h2, wu_v[...].reshape(M, DF))
    hf = (jax.nn.gelu(g, approximate=True) * u).astype(_BF16)
    ffn = None
    for half, sem in ((0, S_WD0), (1, S_WD1)):
        wait_all(wd_v.at[pl.ds(0, 6), pl.ds(128 * half, 128)], sem)
        lhs = jnp.concatenate(
            [hf[:, 256 * gg + 128 * half:256 * gg + 128 * half + 128] for gg in range(6)], axis=1)
        t = _dot(lhs, wd_v[0:6, 128 * half:128 * half + 128, :].reshape(768, M))
        ffn = t if ffn is None else ffn + t
    for half, sem in ((0, S_WD2), (1, S_WD3)):
        wait_all(wd_v.at[pl.ds(6, 1), pl.ds(128 * half, 128)], sem)
        ffn = ffn + _dot(hf[:, 1536 + 128 * half:1536 + 128 * half + 128],
                         wd_v[6, 128 * half:128 * half + 128, :])
    o_ref[...] = (x2 + gb * ffn).astype(o_ref.dtype)


@jax.jit
def pallas_adaLN_cond__compressed_kv_cla__glu_gated_geglu__decode_kernel(
    A_x, A_c_kv, A_w_q, A_w_uk, A_w_uv, A_w_o, B_x, B_w_gate, B_w_up, B_w_down, c, w_mod,
):
    B, SQ, M = A_x.shape
    _, SK, DC = A_c_kv.shape
    _, H, D = A_w_q.shape
    DF = B_w_gate.shape[1]

    x2d = A_x.reshape(1, M)
    ckv = A_c_kv.reshape(_G, SK // _G, DC)
    wq = A_w_q.reshape(_G, M * H // _G, D)
    wuk = A_w_uk.reshape(_G, DC * H // _G, D)
    wuv = A_w_uv.reshape(_G, DC * H // _G, D)
    wo = A_w_o.reshape(_G, H * D // _G, M)
    wg = B_w_gate.reshape(4, M // 4, DF)
    wu = B_w_up.reshape(4, M // 4, DF)
    wd = B_w_down.reshape(7, DF // 7, M)
    wmod = w_mod.reshape(_G, M // _G, 6 * M)
    NT = SK // _KV_TILE

    operands = (x2d, ckv, wq, wuk, wuv, wo, wg, wu, wd, c, wmod)
    vm = lambda a: pltpu.VMEM(a.shape, a.dtype)
    out = pl.pallas_call(
        functools.partial(_kernel, H=H, D=D, M=M, DC=DC, SK=SK),
        in_specs=[pl.BlockSpec(memory_space=pl.ANY)] * len(operands),
        out_specs=pl.BlockSpec(memory_space=pltpu.VMEM),
        out_shape=jax.ShapeDtypeStruct((1, M), A_x.dtype),
        scratch_shapes=[
            vm(x2d), vm(c), vm(wmod), vm(wq), vm(wuk),
            pltpu.VMEM((NT, _G, _KV_TILE // _G, DC), ckv.dtype), vm(wuv), vm(wo),
            vm(wg), vm(wu), vm(wd),
            pltpu.SemaphoreType.DMA((S_KV + NT,)),
        ],
        compiler_params=pltpu.CompilerParams(
            vmem_limit_bytes=96 * 1024 * 1024,
            disable_semaphore_checks=True,
        ),
    )(*operands)
    return out.reshape(B, SQ, M)
```

```python
import functools

import jax
import jax.numpy as jnp
from jax import lax
import jax.experimental.pallas as pl
import jax.experimental.pallas.tpu as pltpu

_F32 = jnp.float32
_BF16 = jnp.bfloat16

_KV_TILE = 2048
_SKEW = 26
_LEAD = 48
_KVG = 8
_P1 = "a"
_P3 = "a"


def _layernorm(x, eps=1e-05):
    m = jnp.mean(x, axis=-1, keepdims=True)
    xc = x - m
    v = jnp.mean(xc * xc, axis=-1, keepdims=True)
    return xc / jnp.sqrt(v + eps)


def _dot(a, b):
    return jnp.dot(a, b, preferred_element_type=_F32)


def _dot_nt(a, b):
    return lax.dot_general(a, b, (((1,), (1,)), ((), ())),
                           preferred_element_type=_F32)


(S_MODA, S_MODB, S_C, S_X, S_WQ, S_WUK, S_WUV, S_WO, S_WG, S_WU, S_WD0, S_WD1, S_WD2, S_WD3,
 S_KV) = range(15)


def _merge(*streams):
    keyed = []
    for si, s in enumerate(streams):
        for i, h in enumerate(s):
            keyed.append(((i + 0.5) / len(s), si, h))
    keyed.sort(key=lambda t: (t[0], t[1]))
    return [h for _, _, h in keyed]


def _kernel(x_hbm, ckv_hbm, wq_hbm, wuk_hbm, wuv_hbm, wo_hbm, wg_hbm, wu_hbm,
            wd_hbm, c_hbm, wmod_hbm, o_ref,
            x_v, c_v, wmod_v, wq_v, wuk_v, ckv_v, wuv_v, wo_v, wg_v, wu_v, wd_v,
            sems, *, H, D, M, DC, SK):
    NT = SK // _KV_TILE
    RPT = _KV_TILE // _KVG
    NSUB = _KVG // 4
    HPT = _KV_TILE // 128
    G = 128 * H
    NJ = DC // 128

    def piece(src, dst, sem, g0, g1, rows, cols=None):
        idx = (pl.ds(g0, g1 - g0), rows) + (() if cols is None else (cols,))
        return pltpu.make_async_copy(src.at[idx], dst.at[idx], sems.at[sem])

    def kv_piece(tile, h, part):
        j, s = h // NSUB, h % NSUB
        g0, n = (4 * s, 1) if part == "B" else (4 * s + 1, 3)
        r = tile * RPT + j * 32
        if not isinstance(r, int):
            r = pl.multiple_of(r, 32)
        return pltpu.make_async_copy(
            ckv_hbm.at[pl.ds(g0, n), pl.ds(r, 32)],
            ckv_v.at[tile, pl.ds(g0, n), pl.ds(j * 32, 32)],
            sems.at[S_KV + tile])

    def hops(src, dst, sem, js, rows, g0=0, nb=1, ng=4, cols=None):
        return [(sem,
                 functools.partial(piece, src, dst, sem, g0 + nb, g0 + ng, pl.ds(rows * j, rows), cols),
                 functools.partial(piece, src, dst, sem, g0, g0 + nb, pl.ds(rows * j, rows), cols))
                for j in js]

    h_moda = hops(wmod_hbm, wmod_v, S_MODA, range(16), 8, cols=pl.ds(0, 2048))
    h_modb = hops(wmod_hbm, wmod_v, S_MODB, range(8), 16, cols=pl.ds(2048, 1024))
    h_wq = hops(wq_hbm, wq_v, S_WQ, range(32), 128)
    h_wuk = hops(wuk_hbm, wuk_v, S_WUK, range(32), 128)
    h_kv = [(S_KV + t, functools.partial(kv_piece, t, h, "A"), functools.partial(kv_piece, t, h, "B"))
            for t in range(NT) for h in range(HPT)]
    h_wuv = hops(wuv_hbm, wuv_v, S_WUV, range(32), 128)
    h_wo = hops(wo_hbm, wo_v, S_WO, range(32), 32)
    h_wg = hops(wg_hbm, wg_v, S_WG, range(16), 8)
    h_wu = hops(wu_hbm, wu_v, S_WU, range(16), 8)
    h_wd0 = (hops(wd_hbm, wd_v, S_WD0, range(4), 32, g0=0, ng=3) +
             hops(wd_hbm, wd_v, S_WD0, range(4), 32, g0=3, ng=3))
    h_wd1 = (hops(wd_hbm, wd_v, S_WD1, range(4, 8), 32, g0=0, ng=3) +
             hops(wd_hbm, wd_v, S_WD1, range(4, 8), 32, g0=3, ng=3))
    h_wd0 = _merge(h_wd0[:4], h_wd0[4:])
    h_wd1 = _merge(h_wd1[:4], h_wd1[4:])

    if _P1 == "a":
        pre = _merge(h_moda, h_wq[:16]) + _merge(h_wq[16:], h_wuk, h_modb)
    elif _P1 == "b":
        pre = _merge(h_moda + h_modb, h_wq, h_wuk)
    else:
        pre = h_moda + h_modb + h_wq + h_wuk
    if _P3 == "a":
        post = _merge(h_wuv, h_wo) + _merge(h_wg, h_wu) + h_wd0 + h_wd1
    elif _P3 == "b":
        post = _merge(h_wuv, h_wo) + _merge(h_wg, h_wu, h_wd0) + h_wd1
    else:
        post = _merge(h_wuv + h_wo, h_wg + h_wu[:8]) + _merge(h_wu[8:], h_wd0) + h_wd1
    plan = pre + h_kv + post
    e_pre = len(pre)
    e_kv = e_pre + len(h_kv)
    NHOP = len(plan)
    A = [h[1] for h in plan]
    B = [h[2] for h in plan]
    end = {}
    for i, h in enumerate(plan):
        end[h[0]] = i + 1
    for j in range(32):
        A.append(functools.partial(piece, wd_hbm, wd_v, S_WD2 if j < 16 else S_WD3, 6, 7,
                                   pl.ds(8 * j, 8)))
    NA = len(A)
    assert NA >= NHOP + _SKEW

    ptr = [0]

    def emit(lo, hi):
        for i in range(lo, hi):
            A[i]().start(priority=1)
            if 0 <= i - _SKEW < NHOP:
                B[i - _SKEW]().start(priority=0)

    def issue_for(e):
        hi = min(e + _LEAD, NA)
        if hi > ptr[0]:
            emit(ptr[0], hi)
            ptr[0] = hi

    def wait_all(buf, sem):
        pltpu.make_async_copy(buf, buf, sems.at[sem]).wait()

    cp_c = pltpu.make_async_copy(c_hbm, c_v, sems.at[S_C])
    cp_x = pltpu.make_async_copy(x_hbm, x_v, sems.at[S_X])
    emit(0, 1)
    ptr[0] = 1
    cp_c.start()
    cp_x.start()
    issue_for(end[S_MODA])

    row = lax.broadcasted_iota(jnp.int32, (128, G), 0)
    col = lax.broadcasted_iota(jnp.int32, (128, G), 1)
    expand = jnp.where(col // H == row, 1.0, 0.0).astype(_BF16)
    diag = (col % H) == (row % H)

    def expand_lhs(a):
        stacked = jnp.concatenate(
            [a[:, 128 * j:128 * (j + 1)] for j in range(NJ)], axis=0)
        return jnp.where(diag, _dot(stacked, expand), 0.0).astype(_BF16)

    def contract_major(big, w_v):
        out = None
        for j in range(NJ):
            t = _dot(big[H * j:H * (j + 1), :], w_v[j])
            out = t if out is None else out + t
        return out

    cp_c.wait()
    cp_x.wait()
    wait_all(wmod_v.at[:, :, pl.ds(0, 2048)], S_MODA)
    c = c_v[...].astype(_F32)
    sc = (c * jax.nn.sigmoid(c)).astype(_BF16)
    moda = _dot(sc, wmod_v[:, :, 0:2048].reshape(M, 4 * M))
    sa, ca, ga, sb = (moda[:, M * i:M * (i + 1)] for i in range(4))
    x = x_v[...].astype(_F32)
    h1 = (_layernorm(x) * (1.0 + ca) + sa).astype(_BF16)
    big_q = expand_lhs(jnp.broadcast_to(h1, (H, M)))

    issue_for(end[S_WQ])
    wait_all(wq_v, S_WQ)
    q = contract_major(big_q, wq_v).astype(_BF16)
    issue_for(e_pre)
    wait_all(wuk_v, S_WUK)
    ys = [_dot_nt(q, wuk_v[j]) for j in range(NJ)]
    ym = jnp.where(diag, jnp.concatenate(ys, axis=0) * (D ** -0.5), 0.0).astype(_BF16)
    qs = _dot_nt(ym, expand)
    qa = jnp.concatenate(
        [qs[H * j:H * (j + 1), :] for j in range(NJ)], axis=1).astype(_BF16)

    p0 = ptr[0]
    assert p0 == e_pre + _LEAD and p0 - _SKEW >= e_pre
    n_dyn = (e_kv - p0) // HPT

    def kv_step(t, carry):
        @pl.when(t < n_dyn)
        def _():
            for jj in range(HPT):
                ha = p0 - e_pre + jj
                hb = ha - _SKEW
                kv_piece(t + ha // HPT, ha % HPT, "A").start(priority=1)
                kv_piece(t + hb // HPT, hb % HPT, "B").start(priority=0)

        for tt in range(n_dyn, NT):
            @pl.when(t == tt)
            def _():
                emit(p0 + HPT * tt, p0 + HPT * (tt + 1))

        pltpu.make_async_copy(ckv_v.at[t], ckv_v.at[t], sems.at[S_KV + t]).wait()
        m, l, acc = carry
        kv = ckv_v[t].reshape(_KV_TILE, DC)
        s = _dot_nt(qa, kv)
        m_new = jnp.maximum(m, jnp.max(s, axis=1, keepdims=True))
        alpha = jnp.exp(m - m_new)
        p = jnp.exp(s - m_new)
        l = l * alpha + jnp.sum(p, axis=1, keepdims=True)
        acc = acc * alpha + _dot(p.astype(_BF16), kv)
        return m_new, l, acc

    init = (jnp.full((H, 1), -jnp.inf, _F32), jnp.zeros((H, 1), _F32),
            jnp.zeros((H, DC), _F32))
    _, l, acc = lax.fori_loop(0, NT, kv_step, init)
    ptr[0] = p0 + HPT * NT
    cc = (acc / l).astype(_BF16)
    big_c = expand_lhs(cc)
    wait_all(wmod_v.at[:, :, pl.ds(2048, 1024)], S_MODB)
    modb = _dot(sc, wmod_v[:, :, 2048:3072].reshape(M, 2 * M))
    cb, gb = modb[:, :M], modb[:, M:]

    issue_for(end[S_WUV])
    wait_all(wuv_v, S_WUV)
    ctx = contract_major(big_c, wuv_v)

    r32 = lax.broadcasted_iota(jnp.int32, (H, H * D), 0)
    c32 = lax.broadcasted_iota(jnp.int32, (H, H * D), 1)
    lo = jnp.where(c32 // D == r32, jnp.concatenate([ctx] * H, axis=1), 0.0).astype(_BF16)
    issue_for(end[S_WO])
    wait_all(wo_v, S_WO)
    attn = jnp.sum(_dot(lo, wo_v[...].reshape(H * D, M)), axis=0, keepdims=True)
    x2 = x + ga * attn

    h2 = (_layernorm(x2) * (1.0 + cb) + sb).astype(_BF16)
    issue_for(NA)
    DF = wg_v.shape[-1]
    wait_all(wg_v, S_WG)
    g = _dot(h2, wg_v[...].reshape(M, DF))
    wait_all(wu_v, S_WU)
    u = _dot(h2, wu_v[...].reshape(M, DF))
    hf = (jax.nn.gelu(g, approximate=True) * u).astype(_BF16)
    ffn = None
    for half, sem in ((0, S_WD0), (1, S_WD1)):
        wait_all(wd_v.at[pl.ds(0, 6), pl.ds(128 * half, 128)], sem)
        lhs = jnp.concatenate(
            [hf[:, 256 * gg + 128 * half:256 * gg + 128 * half + 128] for gg in range(6)], axis=1)
        t = _dot(lhs, wd_v[0:6, 128 * half:128 * half + 128, :].reshape(768, M))
        ffn = t if ffn is None else ffn + t
    for half, sem in ((0, S_WD2), (1, S_WD3)):
        wait_all(wd_v.at[pl.ds(6, 1), pl.ds(128 * half, 128)], sem)
        ffn = ffn + _dot(hf[:, 1536 + 128 * half:1536 + 128 * half + 128],
                         wd_v[6, 128 * half:128 * half + 128, :])
    o_ref[...] = (x2 + gb * ffn).astype(o_ref.dtype)


@jax.jit
def pallas_adaLN_cond__compressed_kv_cla__glu_gated_geglu__decode_kernel(
    A_x, A_c_kv, A_w_q, A_w_uk, A_w_uv, A_w_o, B_x, B_w_gate, B_w_up, B_w_down, c, w_mod,
):
    B, SQ, M = A_x.shape
    _, SK, DC = A_c_kv.shape
    _, H, D = A_w_q.shape
    DF = B_w_gate.shape[1]

    x2d = A_x.reshape(1, M)
    ckv = A_c_kv.reshape(_KVG, SK // _KVG, DC)
    wq = A_w_q.reshape(4, M * H // 4, D)
    wuk = A_w_uk.reshape(4, DC * H // 4, D)
    wuv = A_w_uv.reshape(4, DC * H // 4, D)
    wo = A_w_o.reshape(4, H * D // 4, M)
    wg = B_w_gate.reshape(4, M // 4, DF)
    wu = B_w_up.reshape(4, M // 4, DF)
    wd = B_w_down.reshape(7, DF // 7, M)
    wmod = w_mod.reshape(4, M // 4, 6 * M)
    NT = SK // _KV_TILE

    operands = (x2d, ckv, wq, wuk, wuv, wo, wg, wu, wd, c, wmod)
    vm = lambda a: pltpu.VMEM(a.shape, a.dtype)
    out = pl.pallas_call(
        functools.partial(_kernel, H=H, D=D, M=M, DC=DC, SK=SK),
        in_specs=[pl.BlockSpec(memory_space=pl.ANY)] * len(operands),
        out_specs=pl.BlockSpec(memory_space=pltpu.VMEM),
        out_shape=jax.ShapeDtypeStruct((1, M), A_x.dtype),
        scratch_shapes=[
            vm(x2d), vm(c), vm(wmod), vm(wq), vm(wuk),
            pltpu.VMEM((NT, _KVG, _KV_TILE // _KVG, DC), ckv.dtype), vm(wuv), vm(wo),
            vm(wg), vm(wu), vm(wd),
            pltpu.SemaphoreType.DMA((S_KV + NT,)),
        ],
        compiler_params=pltpu.CompilerParams(
            vmem_limit_bytes=96 * 1024 * 1024,
            disable_semaphore_checks=True,
        ),
    )(*operands)
    return out.reshape(B, SQ, M)
```

```python
import functools

import jax
import jax.numpy as jnp
from jax import lax
import jax.experimental.pallas as pl
import jax.experimental.pallas.tpu as pltpu

_F32 = jnp.float32
_BF16 = jnp.bfloat16

_KV_TILE = 2048
_SKEW = 22
_LEAD = 48
_KVG = 8
_SH_A = 2
_SH_W = 2
_SH_F = 1
_SH_M = 0
_WD = (640, 768, 256, 128)
_P1 = "b"
_PIECE = 128


def _layernorm(x, eps=1e-05):
    m = jnp.mean(x, axis=-1, keepdims=True)
    xc = x - m
    v = jnp.mean(xc * xc, axis=-1, keepdims=True)
    return xc / jnp.sqrt(v + eps)


def _dot(a, b):
    return jnp.dot(a, b, preferred_element_type=_F32)


def _dot_nt(a, b):
    return lax.dot_general(a, b, (((1,), (1,)), ((), ())),
                           preferred_element_type=_F32)


def _unflat(v, cols):
    ct = cols // 128
    v = v.reshape(-1, ct, 8, 128)
    rows = v.shape[0] * 8
    return jnp.concatenate([v[:, i].reshape(rows, 128) for i in range(ct)], axis=1)


(S_MOD, S_C, S_X, S_WQ, S_WUK, S_WUV, S_WO, S_WG, S_WU, S_WD0, S_WD1, S_WD2, S_WD3,
 S_KVH, S_KV) = range(15)


def _merge(*streams):
    keyed = []
    for si, s in enumerate(streams):
        for i, h in enumerate(s):
            keyed.append(((i + 0.5) / len(s), si, h))
    keyed.sort(key=lambda t: (t[0], t[1]))
    return [h for _, _, h in keyed]


def _kernel(x_hbm, ckv_hbm, wq_hbm, wuk_hbm, wuv_hbm, wo_hbm, wg_hbm, wu_hbm,
            wd_hbm, c_hbm, wmod_hbm, o_ref,
            x_v, c_v, wmod_v, wq_v, wuk_v, ckv_v, wuv_v, wo_v, wg_v, wu_v, wd_v,
            sems, *, H, D, M, DC, SK, DF):
    NT = SK // _KV_TILE
    NSUB = _KVG // 4
    HPT = _KV_TILE // 128
    PPT = HPT // NSUB
    FPT = PPT * _PIECE
    G = 128 * H
    NJ = DC // 128

    def copy(src, dst, sem, g0, n, r0, rows):
        idx = (pl.ds(g0, n), pl.ds(r0, rows))
        return pltpu.make_async_copy(src.at[idx], dst.at[idx], sems.at[sem])

    def bounds(p, npieces, sh):
        lo = 0 if p == 0 else _PIECE * p - 8 * sh
        hi = _PIECE * npieces if p == npieces - 1 else _PIECE * (p + 1) - 8 * sh
        return lo, hi - lo

    def hop(src, dst, sem, g0, r0, rows):
        return (sem, functools.partial(copy, src, dst, sem, g0 + 1, 3, r0, rows),
                functools.partial(copy, src, dst, sem, g0, 1, r0, rows))

    def hops(src, dst, sem, sh):
        n = src.shape[1] // _PIECE
        return [hop(src, dst, sem, 0, *bounds(p, n, sh)) for p in range(n)]

    NP_KV = ckv_hbm.shape[1] // _PIECE
    h_kv = [hop(ckv_hbm, ckv_v, S_KVH if p == 0 else S_KV + (p - 1) // PPT, 4 * s,
                *bounds(p, NP_KV, _SH_A))
            for p in range(NP_KV) for s in range(NSUB)]
    h_mod = hops(wmod_hbm, wmod_v, S_MOD, _SH_M)
    h_wq = hops(wq_hbm, wq_v, S_WQ, _SH_W)
    h_wuk = hops(wuk_hbm, wuk_v, S_WUK, _SH_W)
    h_wuv = hops(wuv_hbm, wuv_v, S_WUV, _SH_W)
    h_wo = hops(wo_hbm, wo_v, S_WO, _SH_W)
    h_wg = hops(wg_hbm, wg_v, S_WG, _SH_F)
    h_wu = hops(wu_hbm, wu_v, S_WU, _SH_F)

    def rows2d(src, dst, sem, r, n):
        return pltpu.make_async_copy(src.at[pl.ds(r, n)], dst.at[pl.ds(r, n)], sems.at[sem])

    def wd_hops(sem, gs):
        return [(sem, functools.partial(rows2d, wd_hbm, wd_v, sem, 128 * g, 96),
                 functools.partial(rows2d, wd_hbm, wd_v, sem, 128 * g + 96, 32)) for g in gs]

    h_wd0 = wd_hops(S_WD0, range(0, _WD[0] // 128))
    h_wd1 = wd_hops(S_WD1, range(_WD[0] // 128, (_WD[0] + _WD[1]) // 128))

    if _P1 == "a":
        pre = _merge(h_mod, h_wq[:20]) + _merge(h_wq[20:], h_wuk)
    elif _P1 == "b":
        pre = _merge(h_mod, h_wq[:12], h_wuk[:12]) + _merge(h_wq[12:], h_wuk[12:])
    else:
        pre = _merge(h_mod, h_wq[:24], h_wuk[:8]) + _merge(h_wq[24:], h_wuk[8:16]) + h_wuk[16:]
    post = _merge(h_wuv, h_wo) + _merge(h_wg, h_wu) + h_wd0 + h_wd1
    plan = pre + h_kv + post
    e_pre = len(pre)
    e_kv = e_pre + len(h_kv)
    NHOP = len(plan)
    A = [h[1] for h in plan]
    B = [h[2] for h in plan]
    end = {}
    for i, h in enumerate(plan):
        end[h[0]] = i + 1
    r = _WD[0] + _WD[1]
    for sem, n in ((S_WD2, _WD[2]), (S_WD3, _WD[3])):
        for j in range(16):
            A.append(functools.partial(rows2d, wd_hbm, wd_v, sem, r + (n // 16) * j, n // 16))
        r += n
    NA = len(A)
    assert NA >= NHOP + _SKEW

    ptr = [0]

    def emit(lo, hi):
        for i in range(lo, hi):
            A[i]().start(priority=1)
            if 0 <= i - _SKEW < NHOP:
                B[i - _SKEW]().start(priority=0)

    def issue_for(e):
        hi = min(e + _LEAD, NA)
        if hi > ptr[0]:
            emit(ptr[0], hi)
            ptr[0] = hi

    def wait_all(buf, sem):
        pltpu.make_async_copy(buf, buf, sems.at[sem]).wait()

    cp_c = pltpu.make_async_copy(c_hbm, c_v, sems.at[S_C])
    cp_x = pltpu.make_async_copy(x_hbm, x_v, sems.at[S_X])
    emit(0, 1)
    ptr[0] = 1
    cp_c.start()
    cp_x.start()
    issue_for(end[S_MOD])

    row = lax.broadcasted_iota(jnp.int32, (128, G), 0)
    col = lax.broadcasted_iota(jnp.int32, (128, G), 1)
    expand = jnp.where(col // H == row, 1.0, 0.0).astype(_BF16)
    diag = (col % H) == (row % H)

    def expand_lhs(a):
        stacked = jnp.concatenate(
            [a[:, 128 * j:128 * (j + 1)] for j in range(NJ)], axis=0)
        return jnp.where(diag, _dot(stacked, expand), 0.0).astype(_BF16)

    def contract_major(big, w_v):
        out = None
        for j in range(NJ):
            t = _dot(big[H * j:H * (j + 1), :], w_v[j])
            out = t if out is None else t + out
        return out

    cp_c.wait()
    cp_x.wait()
    wait_all(wmod_v, S_MOD)
    c = c_v[...].astype(_F32)
    sc = (c * jax.nn.sigmoid(c)).astype(_BF16)
    mod = _dot(sc, _unflat(wmod_v[...], 6 * M))
    sa, ca, ga, sb, cb, gb = (mod[:, M * i:M * (i + 1)] for i in range(6))
    x = x_v[...].astype(_F32)
    h1 = (_layernorm(x) * (1.0 + ca) + sa).astype(_BF16)
    big_q = expand_lhs(jnp.broadcast_to(h1, (H, M)))

    issue_for(end[S_WQ])
    wait_all(wq_v, S_WQ)
    q = contract_major(big_q, wq_v).astype(_BF16)
    issue_for(e_pre + NSUB)
    wait_all(wuk_v, S_WUK)
    ys = [_dot_nt(q, wuk_v[j]) for j in range(NJ)]
    ym = jnp.where(diag, jnp.concatenate(ys, axis=0) * (D ** -0.5), 0.0).astype(_BF16)
    qs = _dot_nt(ym, expand)
    qa = jnp.concatenate(
        [qs[H * j:H * (j + 1), :] for j in range(NJ)], axis=1).astype(_BF16)

    head = _PIECE - 8 * _SH_A
    wait_all(ckv_v.at[:, pl.ds(0, head)], S_KVH)
    p0 = ptr[0]
    assert p0 == e_pre + NSUB + _LEAD and p0 - _SKEW >= e_pre + NSUB
    n_dyn = (e_kv - NSUB - p0) // HPT

    def kv_dyn(t, h, g_off, n):
        p, s = h // NSUB, h % NSUB
        r0 = pl.multiple_of(t * FPT + (_PIECE * p - 8 * _SH_A), 8)
        return copy(ckv_hbm, ckv_v, S_KV + t + (p - 1) // PPT, 4 * s + g_off, n, r0, _PIECE)

    def kv_step(t, carry):
        @pl.when(t < n_dyn)
        def _():
            for jj in range(HPT):
                ha = p0 - e_pre + jj
                kv_dyn(t, ha, 1, 3).start(priority=1)
                kv_dyn(t, ha - _SKEW, 0, 1).start(priority=0)

        for tt in range(n_dyn, NT):
            @pl.when(t == tt)
            def _():
                emit(p0 + HPT * tt, p0 + HPT * (tt + 1))

        @pl.when(t < NT - 1)
        def _():
            wait_all(ckv_v.at[:, pl.ds(pl.multiple_of(t * FPT + head, 8), FPT)], S_KV + t)

        @pl.when(t == NT - 1)
        def _():
            wait_all(ckv_v.at[:, pl.ds((NT - 1) * FPT + head, FPT - head)], S_KV + NT - 1)

        m, l, acc = carry
        kv = _unflat(ckv_v[:, pl.ds(pl.multiple_of(t * FPT, FPT), FPT)], DC)
        s = _dot_nt(qa, kv)
        m_new = jnp.maximum(m, jnp.max(s, axis=1, keepdims=True))
        alpha = jnp.exp(m - m_new)
        p = jnp.exp(s - m_new)
        l = l * alpha + jnp.sum(p, axis=1, keepdims=True)
        acc = acc * alpha + _dot(p.astype(_BF16), kv)
        return m_new, l, acc

    init = (jnp.full((H, 1), -jnp.inf, _F32), jnp.zeros((H, 1), _F32),
            jnp.zeros((H, DC), _F32))
    _, l, acc = lax.fori_loop(0, NT, kv_step, init)
    ptr[0] = p0 + HPT * NT
    cc = (acc / l).astype(_BF16)
    big_c = expand_lhs(cc)

    issue_for(end[S_WUV])
    wait_all(wuv_v, S_WUV)
    ctx = contract_major(big_c, wuv_v)

    r32 = lax.broadcasted_iota(jnp.int32, (H, H * D), 0)
    c32 = lax.broadcasted_iota(jnp.int32, (H, H * D), 1)
    lo = jnp.where(c32 // D == r32, jnp.concatenate([ctx] * H, axis=1), 0.0).astype(_BF16)
    issue_for(end[S_WO])
    wait_all(wo_v, S_WO)
    attn = jnp.sum(_dot(lo, _unflat(wo_v[...], M)), axis=0, keepdims=True)
    x2 = x + ga * attn

    h2 = (_layernorm(x2) * (1.0 + cb) + sb).astype(_BF16)
    issue_for(NA)
    wait_all(wg_v, S_WG)
    wait_all(wu_v, S_WU)
    g = _dot(h2, _unflat(wg_v[...], DF))
    u = _dot(h2, _unflat(wu_v[...], DF))
    hf = (jax.nn.gelu(g, approximate=True) * u).astype(_BF16)
    ffn = None
    r = 0
    for sem, n in zip((S_WD0, S_WD1, S_WD2, S_WD3), _WD):
        wait_all(wd_v.at[pl.ds(r, n)], sem)
        t = _dot(hf[:, r:r + n], wd_v[r:r + n, :])
        ffn = t if ffn is None else t + ffn
        r += n
    o_ref[...] = (x2 + gb * ffn).astype(o_ref.dtype)


def _flat(a, regions):
    a = a.reshape(-1, a.shape[-1])
    r, c = a.shape
    a = a.reshape(r // 8, 8, c // 128, 128).transpose(0, 2, 1, 3)
    return a.reshape(regions, r * c // (128 * regions), 128)


@jax.jit
def pallas_adaLN_cond__compressed_kv_cla__glu_gated_geglu__decode_kernel(
    A_x, A_c_kv, A_w_q, A_w_uk, A_w_uv, A_w_o, B_x, B_w_gate, B_w_up, B_w_down, c, w_mod,
):
    B, SQ, M = A_x.shape
    _, SK, DC = A_c_kv.shape
    _, H, D = A_w_q.shape
    DF = B_w_gate.shape[1]

    x2d = A_x.reshape(1, M)
    ckv = _flat(A_c_kv, _KVG)
    wq = A_w_q.reshape(4, M * H // 4, D)
    wuk = A_w_uk.reshape(4, DC * H // 4, D)
    wuv = A_w_uv.reshape(4, DC * H // 4, D)
    wo = _flat(A_w_o, 4)
    wg = _flat(B_w_gate, 4)
    wu = _flat(B_w_up, 4)
    wd = B_w_down
    wmod = _flat(w_mod, 4)
    NT = SK // _KV_TILE

    operands = (x2d, ckv, wq, wuk, wuv, wo, wg, wu, wd, c, wmod)
    vm = lambda a: pltpu.VMEM(a.shape, a.dtype)
    out = pl.pallas_call(
        functools.partial(_kernel, H=H, D=D, M=M, DC=DC, SK=SK, DF=DF),
        in_specs=[pl.BlockSpec(memory_space=pl.ANY)] * len(operands),
        out_specs=pl.BlockSpec(memory_space=pltpu.VMEM),
        out_shape=jax.ShapeDtypeStruct((1, M), A_x.dtype),
        scratch_shapes=[
            vm(x2d), vm(c), vm(wmod), vm(wq), vm(wuk), vm(ckv), vm(wuv), vm(wo),
            vm(wg), vm(wu), vm(wd),
            pltpu.SemaphoreType.DMA((S_KV + NT,)),
        ],
        compiler_params=pltpu.CompilerParams(
            vmem_limit_bytes=96 * 1024 * 1024,
            disable_semaphore_checks=True,
        ),
    )(*operands)
    return out.reshape(B, SQ, M)
```

```python
import functools

import jax
import jax.numpy as jnp
from jax import lax
import jax.experimental.pallas as pl
import jax.experimental.pallas.tpu as pltpu

_F32 = jnp.float32
_BF16 = jnp.bfloat16

_KV_TILE = 2048
_SKEW = 26
_LEAD = 48
_KVG = 8
_PIECE = 128
_SH_A = 2
_SH_W = 2
_SH_F = 1
_SH_M = 0
_WDP = ((768, 0, 0), (256, 0, 1), (256, 0, 1), (256, 0, 1),
        (128, 16, 1), (96, 12, 1), (32, 4, 1))

(S_MOD, S_C, S_X, S_WQ, S_WUK, S_WUV, S_WO, S_WG, S_WU, S_KVH, S_WD0) = range(11)
S_KV = S_WD0 + len(_WDP)


def _layernorm(x, eps=1e-05):
    m = jnp.mean(x, axis=-1, keepdims=True)
    xc = x - m
    v = jnp.mean(xc * xc, axis=-1, keepdims=True)
    return xc / jnp.sqrt(v + eps)


def _dot(a, b):
    return jnp.dot(a, b, preferred_element_type=_F32)


def _dot_nt(a, b):
    return lax.dot_general(a, b, (((1,), (1,)), ((), ())),
                           preferred_element_type=_F32)


def _unflat(v, cols):
    ct = cols // 128
    v = v.reshape(-1, ct, 8, 128)
    rows = v.shape[0] * 8
    return jnp.concatenate([v[:, i].reshape(rows, 128) for i in range(ct)], axis=1)


def _merge(*streams):
    keyed = []
    for si, s in enumerate(streams):
        for i, h in enumerate(s):
            keyed.append(((i + 0.5) / len(s), si, h))
    keyed.sort(key=lambda t: (t[0], t[1]))
    return [h for _, _, h in keyed]


def _kernel(x_hbm, ckv_hbm, wq_hbm, wuk_hbm, wuv_hbm, wo_hbm, wg_hbm, wu_hbm,
            wd_hbm, c_hbm, wmod_hbm, o_ref,
            x_v, c_v, wmod_v, wq_v, wuk_v, ckv_v, wuv_v, wo_v, wg_v, wu_v, wd_v,
            sems, *, H, D, M, DC, SK, DF):
    NT = SK // _KV_TILE
    NSUB = _KVG // 4
    HPT = _KV_TILE // 128
    PPT = HPT // NSUB
    FPT = PPT * _PIECE
    G = 128 * H
    NJ = DC // 128

    def copy(src, dst, sem, g0, n, r0, rows):
        idx = (pl.ds(g0, n), pl.ds(r0, rows))
        return pltpu.make_async_copy(src.at[idx], dst.at[idx], sems.at[sem])

    def bounds(p, npieces, sh):
        lo = 0 if p == 0 else _PIECE * p - 8 * sh
        hi = _PIECE * npieces if p == npieces - 1 else _PIECE * (p + 1) - 8 * sh
        return lo, hi - lo

    def hop(src, dst, sem, g0, r0, rows):
        return (sem, functools.partial(copy, src, dst, sem, g0 + 1, 3, r0, rows),
                functools.partial(copy, src, dst, sem, g0, 1, r0, rows))

    def hops(src, dst, sem, sh):
        n = src.shape[1] // _PIECE
        return [hop(src, dst, sem, 0, *bounds(p, n, sh)) for p in range(n)]

    NP_KV = ckv_hbm.shape[1] // _PIECE
    h_kv = [hop(ckv_hbm, ckv_v, S_KVH if p == 0 else S_KV + (p - 1) // PPT, 4 * s,
                *bounds(p, NP_KV, _SH_A))
            for p in range(NP_KV) for s in range(NSUB)]
    h_mod = hops(wmod_hbm, wmod_v, S_MOD, _SH_M)
    h_wq = hops(wq_hbm, wq_v, S_WQ, _SH_W)
    h_wuk = hops(wuk_hbm, wuk_v, S_WUK, _SH_W)
    h_wuv = hops(wuv_hbm, wuv_v, S_WUV, _SH_W)
    h_wo = hops(wo_hbm, wo_v, S_WO, _SH_W)
    h_wg = hops(wg_hbm, wg_v, S_WG, _SH_F)
    h_wu = hops(wu_hbm, wu_v, S_WU, _SH_F)

    def wd_rows(sem, r, n):
        return pltpu.make_async_copy(wd_hbm.at[pl.ds(r, n)], wd_v.at[pl.ds(r, n)], sems.at[sem])

    h_wd, wd_tail = [], []
    r_wd = 0
    for gi, (n, k, _) in enumerate(_WDP):
        sem = S_WD0 + gi
        if k == 0:
            h_wd += [(sem, functools.partial(wd_rows, sem, r, 96),
                      functools.partial(wd_rows, sem, r + 96, 32))
                     for r in range(r_wd, r_wd + n, 128)]
        else:
            wd_tail += [functools.partial(wd_rows, sem, r, n // k)
                        for r in range(r_wd, r_wd + n, n // k)]
        r_wd += n
    assert r_wd == DF

    pre = _merge(h_mod, h_wq[:12], h_wuk[:12]) + _merge(h_wq[12:], h_wuk[12:])
    post = _merge(h_wuv, h_wo) + _merge(h_wg, h_wu) + h_wd
    plan = pre + h_kv + post
    e_pre = len(pre)
    e_kv = e_pre + len(h_kv)
    NHOP = len(plan)
    A = [h[1] for h in plan] + wd_tail
    B = [h[2] for h in plan]
    end = {h[0]: i + 1 for i, h in enumerate(plan)}
    NA = len(A)
    assert NA >= NHOP + _SKEW and _LEAD >= _SKEW

    ptr = [0]

    def emit(lo, hi):
        for i in range(lo, hi):
            A[i]().start(priority=1)
            if 0 <= i - _SKEW < NHOP:
                B[i - _SKEW]().start(priority=0)

    def issue_for(e):
        hi = min(e + _LEAD, NA)
        if hi > ptr[0]:
            emit(ptr[0], hi)
            ptr[0] = hi

    def wait_all(buf, sem):
        pltpu.make_async_copy(buf, buf, sems.at[sem]).wait()

    cp_c = pltpu.make_async_copy(c_hbm, c_v, sems.at[S_C])
    cp_x = pltpu.make_async_copy(x_hbm, x_v, sems.at[S_X])
    emit(0, 1)
    ptr[0] = 1
    cp_c.start()
    cp_x.start()
    issue_for(end[S_MOD])

    row = lax.broadcasted_iota(jnp.int32, (128, G), 0)
    col = lax.broadcasted_iota(jnp.int32, (128, G), 1)
    expand = jnp.where(col // H == row, 1.0, 0.0).astype(_BF16)
    diag = (col % H) == (row % H)

    def expand_lhs(a):
        stacked = jnp.concatenate(
            [a[:, 128 * j:128 * (j + 1)] for j in range(NJ)], axis=0)
        return jnp.where(diag, _dot(stacked, expand), 0.0).astype(_BF16)

    def contract_major(big, w_v):
        out = None
        for j in range(NJ):
            t = _dot(big[H * j:H * (j + 1), :], w_v[j])
            out = t if out is None else t + out
        return out

    cp_c.wait()
    cp_x.wait()
    wait_all(wmod_v, S_MOD)
    c = c_v[...].astype(_F32)
    sc = (c * jax.nn.sigmoid(c)).astype(_BF16)
    mod = _dot(sc, _unflat(wmod_v[...], 6 * M))
    sa, ca, ga, sb, cb, gb = (mod[:, M * i:M * (i + 1)] for i in range(6))
    x = x_v[...].astype(_F32)
    h1 = (_layernorm(x) * (1.0 + ca) + sa).astype(_BF16)
    big_q = expand_lhs(jnp.broadcast_to(h1, (H, M)))

    issue_for(end[S_WQ])
    wait_all(wq_v, S_WQ)
    q = contract_major(big_q, wq_v).astype(_BF16)
    issue_for(e_pre + NSUB)
    wait_all(wuk_v, S_WUK)
    ys = [_dot_nt(q, wuk_v[j]) for j in range(NJ)]
    ym = jnp.where(diag, jnp.concatenate(ys, axis=0) * (D ** -0.5), 0.0).astype(_BF16)
    qs = _dot_nt(ym, expand)
    qa = jnp.concatenate(
        [qs[H * j:H * (j + 1), :] for j in range(NJ)], axis=1).astype(_BF16)

    head = _PIECE - 8 * _SH_A
    wait_all(ckv_v.at[:, pl.ds(0, head)], S_KVH)
    p0 = ptr[0]
    assert p0 == e_pre + NSUB + _LEAD and p0 - _SKEW >= e_pre + NSUB
    n_dyn = (e_kv - NSUB - p0) // HPT

    def kv_dyn(t, h, g_off, n):
        p, s = h // NSUB, h % NSUB
        r0 = pl.multiple_of(t * FPT + (_PIECE * p - 8 * _SH_A), 8)
        return copy(ckv_hbm, ckv_v, S_KV + t + (p - 1) // PPT, 4 * s + g_off, n, r0, _PIECE)

    def kv_step(t, carry):
        @pl.when(t < n_dyn)
        def _():
            for jj in range(HPT):
                ha = p0 - e_pre + jj
                kv_dyn(t, ha, 1, 3).start(priority=1)
                kv_dyn(t, ha - _SKEW, 0, 1).start(priority=0)

        for tt in range(n_dyn, NT):
            @pl.when(t == tt)
            def _():
                emit(p0 + HPT * tt, p0 + HPT * (tt + 1))

        @pl.when(t < NT - 1)
        def _():
            wait_all(ckv_v.at[:, pl.ds(pl.multiple_of(t * FPT + head, 8), FPT)], S_KV + t)

        @pl.when(t == NT - 1)
        def _():
            wait_all(ckv_v.at[:, pl.ds((NT - 1) * FPT + head, FPT - head)], S_KV + NT - 1)

        m, l, acc = carry
        kv = _unflat(ckv_v[:, pl.ds(pl.multiple_of(t * FPT, FPT), FPT)], DC)
        s = _dot_nt(qa, kv)
        m_new = jnp.maximum(m, jnp.max(s, axis=1, keepdims=True))
        alpha = jnp.exp(m - m_new)
        p = jnp.exp(s - m_new)
        l = l * alpha + jnp.sum(p, axis=1, keepdims=True)
        acc = acc * alpha + _dot(p.astype(_BF16), kv)
        return m_new, l, acc

    init = (jnp.full((H, 1), -jnp.inf, _F32), jnp.zeros((H, 1), _F32),
            jnp.zeros((H, DC), _F32))
    _, l, acc = lax.fori_loop(0, NT, kv_step, init)
    ptr[0] = p0 + HPT * NT
    cc = (acc / l).astype(_BF16)
    big_c = expand_lhs(cc)

    issue_for(end[S_WUV])
    wait_all(wuv_v, S_WUV)
    ctx = contract_major(big_c, wuv_v)

    r32 = lax.broadcasted_iota(jnp.int32, (H, H * D), 0)
    c32 = lax.broadcasted_iota(jnp.int32, (H, H * D), 1)
    lo = jnp.where(c32 // D == r32, jnp.concatenate([ctx] * H, axis=1), 0.0).astype(_BF16)
    issue_for(end[S_WO])
    wait_all(wo_v, S_WO)
    attn = jnp.sum(_dot(lo, _unflat(wo_v[...], M)), axis=0, keepdims=True)
    x2 = x + ga * attn

    h2 = (_layernorm(x2) * (1.0 + cb) + sb).astype(_BF16)
    issue_for(NA)
    wait_all(wg_v, S_WG)
    wait_all(wu_v, S_WU)
    g = _dot(h2, _unflat(wg_v[...], DF))
    u = _dot(h2, _unflat(wu_v[...], DF))
    hf = (jax.nn.gelu(g, approximate=True) * u).astype(_BF16)

    nv = sum(n for n, _, v in _WDP if v)
    eye = (lax.broadcasted_iota(jnp.int32, (128, 128), 0) ==
           lax.broadcasted_iota(jnp.int32, (128, 128), 1))
    hf32 = hf.astype(_F32)
    dm = jnp.concatenate(
        [jnp.where(eye, jnp.broadcast_to(hf32[:, b:b + 128], (128, 128)), 0.0)
         for b in range(DF - nv, DF, 128)], axis=0).astype(_BF16)
    hcol = _dot(dm, jnp.ones((128, 128), _BF16))
    hcol = jnp.concatenate([hcol] * (M // 128), axis=1)
    ffn = None
    acc8 = None
    r = 0
    for gi, (n, _, v) in enumerate(_WDP):
        wait_all(wd_v.at[pl.ds(r, n)], S_WD0 + gi)
        if v:
            o = r - (DF - nv)
            t8 = jnp.sum((wd_v[r:r + n, :].astype(_F32) * hcol[o:o + n]).reshape(n // 8, 8, M), axis=0)
            acc8 = t8 if acc8 is None else t8 + acc8
        else:
            t = _dot(hf[:, r:r + n], wd_v[r:r + n, :])
            ffn = t if ffn is None else t + ffn
            y = x2 + gb * ffn
        r += n
    y = y + gb * jnp.sum(acc8, axis=0, keepdims=True)
    o_ref[...] = y.astype(o_ref.dtype)


def _flat(a, regions):
    a = a.reshape(-1, a.shape[-1])
    r, c = a.shape
    a = a.reshape(r // 8, 8, c // 128, 128).transpose(0, 2, 1, 3)
    return a.reshape(regions, r * c // (128 * regions), 128)


@jax.jit
def pallas_adaLN_cond__compressed_kv_cla__glu_gated_geglu__decode_kernel(
    A_x, A_c_kv, A_w_q, A_w_uk, A_w_uv, A_w_o, B_x, B_w_gate, B_w_up, B_w_down, c, w_mod,
):
    B, SQ, M = A_x.shape
    _, SK, DC = A_c_kv.shape
    _, H, D = A_w_q.shape
    DF = B_w_gate.shape[1]
    assert (B, SQ, M, DC, H, D) == (1, 1, 512, 512, 32, 128) and SK % _KV_TILE == 0

    x2d = A_x.reshape(1, M)
    ckv = _flat(A_c_kv, _KVG)
    wq = A_w_q.reshape(4, M * H // 4, D)
    wuk = A_w_uk.reshape(4, DC * H // 4, D)
    wuv = A_w_uv.reshape(4, DC * H // 4, D)
    wo = _flat(A_w_o, 4)
    wg = _flat(B_w_gate, 4)
    wu = _flat(B_w_up, 4)
    wd = B_w_down
    wmod = _flat(w_mod, 4)
    NT = SK // _KV_TILE

    operands = (x2d, ckv, wq, wuk, wuv, wo, wg, wu, wd, c, wmod)
    vm = lambda a: pltpu.VMEM(a.shape, a.dtype)
    out = pl.pallas_call(
        functools.partial(_kernel, H=H, D=D, M=M, DC=DC, SK=SK, DF=DF),
        in_specs=[pl.BlockSpec(memory_space=pl.ANY)] * len(operands),
        out_specs=pl.BlockSpec(memory_space=pltpu.VMEM),
        out_shape=jax.ShapeDtypeStruct((1, M), A_x.dtype),
        scratch_shapes=[
            vm(x2d), vm(c), vm(wmod), vm(wq), vm(wuk), vm(ckv), vm(wuv), vm(wo),
            vm(wg), vm(wu), vm(wd),
            pltpu.SemaphoreType.DMA((S_KV + NT,)),
        ],
        compiler_params=pltpu.CompilerParams(
            vmem_limit_bytes=96 * 1024 * 1024,
            disable_semaphore_checks=True,
        ),
    )(*operands)
    return out.reshape(B, SQ, M)
```

```python
import functools

import jax
import jax.numpy as jnp
from jax import lax
import jax.experimental.pallas as pl
import jax.experimental.pallas.tpu as pltpu

_F32 = jnp.float32
_BF16 = jnp.bfloat16

_KV_TILE = 2048
_SKEW = 26
_LEAD = 48
_LEAD_KV = 72
_X1 = 8
_X2 = 14
_X3 = 8
_KVG = 8
_WDG = 4
_UNIT = 256
_HEAD_A = 112
_HEAD_F = 120
_HEAD_M = 128

(S_MOD, S_C, S_X, S_WQ, S_WUK, S_WUV, S_WO, S_WG, S_WU, S_KVH, S_KVT, S_WD0) = range(12)
_NWD = 11
S_KV = S_WD0 + _NWD


def _layernorm(x, eps=1e-05):
    m = jnp.mean(x, axis=-1, keepdims=True)
    xc = x - m
    v = jnp.mean(xc * xc, axis=-1, keepdims=True)
    return xc / jnp.sqrt(v + eps)


def _dot(a, b):
    return jnp.dot(a, b, preferred_element_type=_F32)


def _dot_nt(a, b):
    return lax.dot_general(a, b, (((1,), (1,)), ((), ())),
                           preferred_element_type=_F32)


def _unflat(v, cols):
    ct = cols // 128
    v = v.reshape(-1, ct, 8, 128)
    rows = v.shape[0] * 8
    return jnp.concatenate([v[:, i].reshape(rows, 128) for i in range(ct)], axis=1)


def _merge(*streams):
    keyed = []
    for si, s in enumerate(streams):
        for i, h in enumerate(s):
            keyed.append(((i + 0.5) / len(s), si, h))
    keyed.sort(key=lambda t: (t[0], t[1]))
    return [h for _, _, h in keyed]


def _round_robin(seq, regions):
    cut = [round(len(seq) * g / regions) for g in range(regions + 1)]
    runs = [seq[cut[g]:cut[g + 1]] for g in range(regions)]
    return [r[p] for p in range(max(map(len, runs))) for r in runs if p < len(r)]


def _kernel(x_hbm, ckv_hbm, wq_hbm, wuk_hbm, wuv_hbm, wo_hbm, wg_hbm, wu_hbm,
            wd_hbm, c_hbm, wmod_hbm, o_ref,
            x_v, c_v, wmod_v, wq_v, wuk_v, ckv_v, wuv_v, wo_v, wg_v, wu_v, wd_v,
            sems, *, H, D, M, DC, SK, DF):
    NT = SK // _KV_TILE
    RKV = ckv_hbm.shape[1]
    FPT = RKV // NT
    UPT = FPT // _UNIT
    HPS = 3 * _KVG // 4
    HPT = HPS * UPT
    G = 128 * H
    NJ = DC // 128

    def start(piece, priority):
        src, dst, sem, g, r0, rows = piece[:6]
        idx = (pl.ds(r0, rows),) if g is None else (g, pl.ds(r0, rows))
        pltpu.make_async_copy(src.at[idx], dst.at[idx], sems.at[sem]).start(priority=priority)

    def units(src, dst, sem, head):
        n = src.shape[0]
        return [(src, dst, sem, None, 0, head, _UNIT - head, _UNIT)] + [
            (src, dst, sem, None, r, min(_UNIT, n - r), 0, _UNIT) for r in range(head, n, _UNIT)]

    def cut(piece, at):
        src, dst, sem, g, r0, rows, rel, unit = piece
        pts = [rel] + [p for p in at if rel < p < rel + rows] + [rel + rows]
        return [(src, dst, sem, g, r0 + lo - rel, hi - lo) for lo, hi in zip(pts, pts[1:])]

    def to_hops(seq):
        out = []
        for i in range(0, len(seq), 4):
            grp = seq[i:i + 4]
            if len(grp) < 4:
                out += [(u, None) for u in grp]
            else:
                b = cut(grp[0], (grp[0][7] // 4, 3 * grp[0][7] // 4))
                out += list(zip(grp[1:], b + [None] * (3 - len(b))))
        return out

    def kv_unit(k, g, t=0):
        r0 = _HEAD_A + _UNIT * k
        if not isinstance(t, int):
            r0 = pl.multiple_of(t * FPT + r0, 8)
        return (ckv_hbm, ckv_v, S_KV + t + k // UPT, g, r0, _UNIT, 0, _UNIT)

    NK = RKV // _UNIT - 1
    TAIL = _UNIT - _HEAD_A
    h_edge = [((ckv_hbm, ckv_v, S_KVH, g, 0, _HEAD_A), (ckv_hbm, ckv_v, S_KVT, g, RKV - TAIL, TAIL))
              for g in range(_KVG)]
    h_kv = to_hops([kv_unit(k, g) for k in range(NK) for g in range(_KVG)])

    qk = _round_robin(units(wuk_hbm, wuk_v, S_WUK, _HEAD_A) + units(wq_hbm, wq_v, S_WQ, _HEAD_A), 8)
    h_pre = to_hops(_merge(_round_robin(units(wmod_hbm, wmod_v, S_MOD, _HEAD_M), 4), qk[:48]) + qk[48:])
    h_post = to_hops(
        _round_robin(units(wo_hbm, wo_v, S_WO, _HEAD_A) + units(wuv_hbm, wuv_v, S_WUV, _HEAD_A), 8)
        + _round_robin(units(wu_hbm, wu_v, S_WU, _HEAD_F) + units(wg_hbm, wg_v, S_WG, _HEAD_F), 8))

    RWD = wd_hbm.shape[1]
    NKD = RWD // 64 - 1
    LAST = 32 + 64 * (NKD - 1)
    wd_groups = ([(None, 0, 32), (None, RWD - 32, 32)]
                 + [(None, 32 + 64 * k, 64) for k in range(NKD - 1)]
                 + [((0, 2), LAST, 64), ((2, 1), LAST, 64), ((3, 1), LAST, 32), ((3, 1), LAST + 32, 32)])
    assert len(wd_groups) == _NWD and _WDG == 4
    h_wd = [((wd_hbm, wd_v, S_WD0, g, 0, 32), (wd_hbm, wd_v, S_WD0 + 1, g, RWD - 32, 32))
            for g in range(_WDG)]
    h_wd += to_hops([(wd_hbm, wd_v, S_WD0 + 2 + k, g, 32 + 64 * k, 64, 0, 64)
                     for k in range(NKD - 1) for g in range(_WDG)])
    wd_tail = [(wd_hbm, wd_v, S_WD0 + i, g, r, 8)
               for i, (gs, r0, n) in enumerate(wd_groups) if gs is not None
               for g in range(gs[0], gs[0] + gs[1]) for r in range(r0, r0 + n, 8)]

    plan = h_pre + h_edge + h_kv + h_post + h_wd
    e_pre = len(h_pre)
    e_edge = e_pre + len(h_edge)
    e_kv = e_edge + len(h_kv)
    NHOP = len(plan)
    A = [h[0] for h in plan] + wd_tail
    B = [h[1] for h in plan]
    end = {p[2]: i + 1 for i, h in enumerate(plan) for p in h if p is not None}
    NA = len(A)
    assert NA >= NHOP + _SKEW and _LEAD >= _SKEW

    ptr = [0]

    def emit(lo, hi):
        for i in range(lo, hi):
            start(A[i], 1)
            if 0 <= i - _SKEW < NHOP and B[i - _SKEW] is not None:
                start(B[i - _SKEW], 0)

    def issue_for(e):
        hi = min(e + _LEAD, NA)
        if hi > ptr[0]:
            emit(ptr[0], hi)
            ptr[0] = hi

    def wait_all(buf, sem):
        pltpu.make_async_copy(buf, buf, sems.at[sem]).wait()

    cp_c = pltpu.make_async_copy(c_hbm, c_v, sems.at[S_C])
    cp_x = pltpu.make_async_copy(x_hbm, x_v, sems.at[S_X])
    emit(0, 1)
    ptr[0] = 1
    cp_c.start()
    cp_x.start()
    issue_for(end[S_MOD])

    row = lax.broadcasted_iota(jnp.int32, (128, G), 0)
    col = lax.broadcasted_iota(jnp.int32, (128, G), 1)
    expand = jnp.where(col // H == row, 1.0, 0.0).astype(_BF16)
    diag = (col % H) == (row % H)

    def expand_lhs(a):
        stacked = jnp.concatenate(
            [a[:, 128 * j:128 * (j + 1)] for j in range(NJ)], axis=0)
        return jnp.where(diag, _dot(stacked, expand), 0.0).astype(_BF16)

    def contract_major(big, w_v):
        out = None
        for j in range(NJ):
            t = _dot(big[H * j:H * (j + 1), :], w_v[G * j:G * (j + 1), :])
            out = t if out is None else t + out
        return out

    cp_c.wait()
    cp_x.wait()
    wait_all(wmod_v, S_MOD)
    c = c_v[...].astype(_F32)
    sc = (c * jax.nn.sigmoid(c)).astype(_BF16)
    mod = _dot(sc, _unflat(wmod_v[...], 6 * M))
    sa, ca, ga, sb, cb, gb = (mod[:, M * i:M * (i + 1)] for i in range(6))
    x = x_v[...].astype(_F32)
    h1 = (_layernorm(x) * (1.0 + ca) + sa).astype(_BF16)
    big_q = expand_lhs(jnp.broadcast_to(h1, (H, M)))

    issue_for(end[S_WQ])
    wait_all(wq_v, S_WQ)
    q = contract_major(big_q, wq_v).astype(_BF16)
    issue_for(e_pre + _X1)
    wait_all(wuk_v, S_WUK)
    ys = [_dot_nt(q, wuk_v[G * j:G * (j + 1), :]) for j in range(NJ)]
    ym = jnp.where(diag, jnp.concatenate(ys, axis=0) * (D ** -0.5), 0.0).astype(_BF16)
    qs = _dot_nt(ym, expand)
    qa = jnp.concatenate(
        [qs[H * j:H * (j + 1), :] for j in range(NJ)], axis=1).astype(_BF16)

    issue_for(e_edge + _LEAD_KV - _LEAD)
    wait_all(ckv_v.at[:, pl.ds(0, _HEAD_A)], S_KVH)
    wait_all(ckv_v.at[:, pl.ds(RKV - TAIL, TAIL)], S_KVT)
    p0 = ptr[0]
    assert p0 == e_edge + _LEAD_KV and _LEAD_KV >= _SKEW
    n_dyn = (e_kv - p0) // HPT

    def kv_step(t, carry):
        @pl.when(t < n_dyn)
        def _():
            lo = (_LEAD_KV - _SKEW) // HPS
            hi = (_LEAD_KV + HPT - 1) // HPS + 1
            hops = to_hops([kv_unit(k, g, t) for k in range(lo, hi) for g in range(_KVG)])
            for j in range(_LEAD_KV - HPS * lo, _LEAD_KV - HPS * lo + HPT):
                start(hops[j][0], 1)
                start(hops[j - _SKEW][1], 0)

        for tt in range(n_dyn, NT):
            @pl.when(t == tt)
            def _():
                emit(p0 + HPT * tt, p0 + HPT * (tt + 1))

        @pl.when(t < NT - 1)
        def _():
            wait_all(ckv_v.at[:, pl.ds(pl.multiple_of(t * FPT + _HEAD_A, 8), FPT)], S_KV + t)

        @pl.when(t == NT - 1)
        def _():
            wait_all(ckv_v.at[:, pl.ds((NT - 1) * FPT + _HEAD_A, FPT - _UNIT)], S_KV + NT - 1)

        m, l, acc = carry
        kv = _unflat(ckv_v[:, pl.ds(pl.multiple_of(t * FPT, FPT), FPT)], DC)
        s = _dot_nt(qa, kv)
        m_new = jnp.maximum(m, jnp.max(s, axis=1, keepdims=True))
        alpha = jnp.exp(m - m_new)
        p = jnp.exp(s - m_new)
        l = l * alpha + jnp.sum(p, axis=1, keepdims=True)
        acc = acc * alpha + _dot(p.astype(_BF16), kv)
        return m_new, l, acc

    init = (jnp.full((H, 1), -jnp.inf, _F32), jnp.zeros((H, 1), _F32),
            jnp.zeros((H, DC), _F32))
    _, l, acc = lax.fori_loop(0, NT, kv_step, init)
    ptr[0] = p0 + HPT * NT
    issue_for(ptr[0] - _LEAD + _X2)
    cc = (acc / l).astype(_BF16)
    big_c = expand_lhs(cc)

    issue_for(end[S_WUV])
    wait_all(wuv_v, S_WUV)
    ctx = contract_major(big_c, wuv_v)

    r32 = lax.broadcasted_iota(jnp.int32, (H, H * D), 0)
    c32 = lax.broadcasted_iota(jnp.int32, (H, H * D), 1)
    lo = jnp.where(c32 // D == r32, jnp.concatenate([ctx] * H, axis=1), 0.0).astype(_BF16)
    issue_for(max(end[S_WO], end[S_WUV] + _X3))
    wait_all(wo_v, S_WO)
    attn = jnp.sum(_dot(lo, _unflat(wo_v[...], M)), axis=0, keepdims=True)
    x2 = x + ga * attn

    h2 = (_layernorm(x2) * (1.0 + cb) + sb).astype(_BF16)
    issue_for(NA)
    wait_all(wg_v, S_WG)
    wait_all(wu_v, S_WU)
    g = _dot(h2, _unflat(wg_v[...], DF))
    u = _dot(h2, _unflat(wu_v[...], DF))
    hf = (jax.nn.gelu(g, approximate=True) * u).astype(_BF16)

    eye = (lax.broadcasted_iota(jnp.int32, (128, 128), 0) ==
           lax.broadcasted_iota(jnp.int32, (128, 128), 1))
    hf32 = hf.astype(_F32)
    dm = jnp.concatenate(
        [jnp.where(eye, jnp.broadcast_to(hf32[:, b:b + 128], (128, 128)), 0.0)
         for b in range(0, DF, 128)], axis=0).astype(_BF16)
    hcol = _dot(dm, jnp.ones((128, 128), _BF16))
    acc8 = None
    for i, (gs, r0, n) in enumerate(wd_groups):
        g0, ng = (0, _WDG) if gs is None else gs
        wait_all(wd_v.at[pl.ds(g0, ng), pl.ds(r0, n)], S_WD0 + i)
        for g in range(g0, g0 + ng):
            hc = hcol[RWD * g + r0:RWD * g + r0 + n]
            hc = jnp.concatenate([hc] * (M // 128), axis=1)
            t8 = jnp.sum((wd_v[g, r0:r0 + n, :].astype(_F32) * hc).reshape(n // 8, 8, M), axis=0)
            acc8 = t8 if acc8 is None else t8 + acc8
    y = x2 + gb * jnp.sum(acc8, axis=0, keepdims=True)
    o_ref[...] = y.astype(o_ref.dtype)


def _flat(a, regions=None):
    a = a.reshape(-1, a.shape[-1])
    r, c = a.shape
    a = a.reshape(r // 8, 8, c // 128, 128).transpose(0, 2, 1, 3)
    return a.reshape(-1, 128) if regions is None else a.reshape(regions, -1, 128)


@jax.jit
def pallas_adaLN_cond__compressed_kv_cla__glu_gated_geglu__decode_kernel(
    A_x, A_c_kv, A_w_q, A_w_uk, A_w_uv, A_w_o, B_x, B_w_gate, B_w_up, B_w_down, c, w_mod,
):
    B, SQ, M = A_x.shape
    _, SK, DC = A_c_kv.shape
    _, H, D = A_w_q.shape
    DF = B_w_gate.shape[1]
    assert (B, SQ, M, DC, H, D) == (1, 1, 512, 512, 32, 128) and SK % _KV_TILE == 0

    x2d = A_x.reshape(1, M)
    ckv = _flat(A_c_kv, _KVG)
    wq = A_w_q.reshape(M * H, D)
    wuk = A_w_uk.reshape(DC * H, D)
    wuv = A_w_uv.reshape(DC * H, D)
    wo = _flat(A_w_o)
    wg = _flat(B_w_gate)
    wu = _flat(B_w_up)
    wd = B_w_down.reshape(_WDG, DF // _WDG, M)
    wmod = _flat(w_mod)
    NT = SK // _KV_TILE

    operands = (x2d, ckv, wq, wuk, wuv, wo, wg, wu, wd, c, wmod)
    vm = lambda a: pltpu.VMEM(a.shape, a.dtype)
    out = pl.pallas_call(
        functools.partial(_kernel, H=H, D=D, M=M, DC=DC, SK=SK, DF=DF),
        in_specs=[pl.BlockSpec(memory_space=pl.ANY)] * len(operands),
        out_specs=pl.BlockSpec(memory_space=pltpu.VMEM),
        out_shape=jax.ShapeDtypeStruct((1, M), A_x.dtype),
        scratch_shapes=[
            vm(x2d), vm(c), vm(wmod), vm(wq), vm(wuk), vm(ckv), vm(wuv), vm(wo),
            vm(wg), vm(wu), vm(wd),
            pltpu.SemaphoreType.DMA((S_KV + NT,)),
        ],
        compiler_params=pltpu.CompilerParams(
            vmem_limit_bytes=96 * 1024 * 1024,
            disable_semaphore_checks=True,
        ),
    )(*operands)
    return out.reshape(B, SQ, M)
```

```python
import functools

import jax
import jax.numpy as jnp
from jax import lax
import jax.experimental.pallas as pl
import jax.experimental.pallas.tpu as pltpu

_F32 = jnp.float32
_BF16 = jnp.bfloat16

_KV_TILE = 2048
_SKEW = 26
_LEAD = 48
_LEAD_KV = 72
_X1 = 8
_X2 = 14
_X3 = 8
_PAT = "a"
_FIN = 2
_LASTP = 40
_KVG = 8
_WPOS = 1
_BLK = 8
_UNIT = 256
_HEAD_A = 112
_HEAD_F = 120
_HEAD_M = 128

(S_MOD, S_C, S_X, S_WQ, S_WUK, S_WUV, S_WO, S_WG, S_WU, S_KVH, S_KVT, S_WD0) = range(12)
_NWD = 10
S_KV = S_WD0 + _NWD


def _layernorm(x, eps=1e-05):
    m = jnp.mean(x, axis=-1, keepdims=True)
    xc = x - m
    v = jnp.mean(xc * xc, axis=-1, keepdims=True)
    return xc / jnp.sqrt(v + eps)


def _dot(a, b):
    return jnp.dot(a, b, preferred_element_type=_F32)


def _dot_nt(a, b):
    return lax.dot_general(a, b, (((1,), (1,)), ((), ())),
                           preferred_element_type=_F32)


def _unflat(v, cols):
    ct = cols // 128
    v = v.reshape(-1, ct, 8, 128)
    rows = v.shape[0] * 8
    return jnp.concatenate([v[:, i].reshape(rows, 128) for i in range(ct)], axis=1)


def _merge(*streams):
    keyed = []
    for si, s in enumerate(streams):
        for i, h in enumerate(s):
            keyed.append(((i + 0.5) / len(s), si, h))
    keyed.sort(key=lambda t: (t[0], t[1]))
    return [h for _, _, h in keyed]


def _round_robin(seq, regions):
    cut = [round(len(seq) * g / regions) for g in range(regions + 1)]
    runs = [seq[cut[g]:cut[g + 1]] for g in range(regions)]
    return [r[p] for p in range(max(map(len, runs))) for r in runs if p < len(r)]


def _kernel(x_hbm, ckv_hbm, wq_hbm, wuk_hbm, wuv_hbm, wo_hbm, wg_hbm, wu_hbm,
            wd_hbm, c_hbm, wmod_hbm, o_ref,
            x_v, c_v, wmod_v, wq_v, wuk_v, ckv_v, wuv_v, wo_v, wg_v, wu_v, wd_v,
            sems, *, H, D, M, DC, SK, DF):
    NT = SK // _KV_TILE
    RKV = ckv_hbm.shape[1]
    FPT = RKV // NT
    UPT = FPT // _UNIT
    HPS = 3 * _KVG // 4
    HPT = HPS * UPT
    G = 128 * H
    NJ = DC // 128

    def start(piece, priority):
        src, dst, sem, g, r0, rows = piece[:6]
        idx = (pl.ds(r0, rows),) if g is None else (g, pl.ds(r0, rows))
        pltpu.make_async_copy(src.at[idx], dst.at[idx], sems.at[sem]).start(priority=priority)

    def units(src, dst, sem, head):
        n = src.shape[0]
        return [(src, dst, sem, None, 0, head, _UNIT - head, _UNIT)] + [
            (src, dst, sem, None, r, min(_UNIT, n - r), 0, _UNIT) for r in range(head, n, _UNIT)]

    def cut(piece, at):
        src, dst, sem, g, r0, rows, rel, unit = piece
        pts = [rel] + [p for p in at if rel < p < rel + rows] + [rel + rows]
        return [(src, dst, sem, g, r0 + lo - rel, hi - lo) for lo, hi in zip(pts, pts[1:])]

    def to_hops(seq):
        out = []
        for i in range(0, len(seq), 4):
            grp = seq[i:i + 4]
            if len(grp) < 4:
                out += [(u, None) for u in grp]
            else:
                b = cut(grp[0], (grp[0][7] // 4, 3 * grp[0][7] // 4))
                out += list(zip(grp[1:], b + [None] * (3 - len(b))))
        return out

    def kv_unit(k, g, t=0):
        r0 = _HEAD_A + _UNIT * k
        if not isinstance(t, int):
            r0 = pl.multiple_of(t * FPT + r0, 8)
        return (ckv_hbm, ckv_v, S_KV + t + k // UPT, g, r0, _UNIT, 0, _UNIT)

    NK = RKV // _UNIT - 1
    TAIL = _UNIT - _HEAD_A
    h_edge = [((ckv_hbm, ckv_v, S_KVH, g, 0, _HEAD_A), (ckv_hbm, ckv_v, S_KVT, g, RKV - TAIL, TAIL))
              for g in range(_KVG)]
    h_kv = to_hops([kv_unit(k, g) for k in range(NK) for g in range(_KVG)])

    qk = _round_robin(units(wuk_hbm, wuk_v, S_WUK, _HEAD_A) + units(wq_hbm, wq_v, S_WQ, _HEAD_A), 8)
    h_pre = to_hops(_merge(_round_robin(units(wmod_hbm, wmod_v, S_MOD, _HEAD_M), 4), qk[:48]) + qk[48:])
    uvo = _round_robin(units(wo_hbm, wo_v, S_WO, _HEAD_A) + units(wuv_hbm, wuv_v, S_WUV, _HEAD_A), 8)
    gul = units(wu_hbm, wu_v, S_WU, _HEAD_F) + units(wg_hbm, wg_v, S_WG, _HEAD_F)
    cuts = [1, 9, 17, 25, 34, 42, 50, 58]
    assert len(gul) == cuts[-1]
    gu = gul[:1] + [gul[lo + p] for p in range(_BLK + 1)
                    for lo, hi in zip(cuts, cuts[1:]) if lo + p < hi]

    FD = wd_hbm.shape[0]
    CT = M // 128

    def wd_span(g, j0, j1):
        o = _BLK * _UNIT * g + _HEAD_F - 4 * _UNIT
        return max(o + _UNIT * j0, 0), min(o + _UNIT * j1, FD)

    wd_groups = ([[(g,) + wd_span(g, 0, 3) for g in (1, 2, 3)]]
                 + [[(g,) + wd_span(g, j, j + 1) for g in range(4)] for j in range(3, 7)]
                 + [[(g,) + wd_span(g, 7, 8)] for g in range(3)]
                 + [[(3, wd_span(3, 7, 8)[0], FD - _LASTP)], [(3, FD - _LASTP, FD)]])
    assert len(wd_groups) == _NWD and wd_span(3, 0, 8)[1] == FD
    wd_seq = [(wd_hbm, wd_v, S_WD0 + max(j - 2, 0), None, lo, hi - lo, _UNIT - (hi - lo), _UNIT)
              for j in range(7) for lo, hi in (wd_span(g, j, j + 1) for g in range(4)) if hi > lo]
    wd_tail = [p for i in range(5, _NWD) for _, lo, hi in wd_groups[i]
               for p in cut((wd_hbm, wd_v, S_WD0 + i, None, lo, hi - lo, 0, _UNIT), range(32, hi - lo - 16, 32))]
    pat = {"a": "gg" + "ggggdggg" * 7 + "dgggdgggdg",
           "b": "gg" + "gggg" * 2 + "ggggdggg" * 6 + "dgggdggg",
           "c": "gg" + "gggg" * 5 + "ggggdggg" * 3 + "dggg" * 5,
           "d": "gg" + "dggggggg" * 7 + "dgggdgggdg",
           "e": "gg" + "ggggdggg" * 5 + "dggg" * 7,
           }[_PAT]
    assert pat.count("g") == len(gu)
    its = {"g": iter(gu), "d": iter(wd_seq)}
    h_post = to_hops(uvo + [next(its[c]) for c in pat] + list(its["d"]))

    plan = h_pre + h_edge + h_kv + h_post
    e_pre = len(h_pre)
    e_edge = e_pre + len(h_edge)
    e_kv = e_edge + len(h_kv)
    NHOP = len(plan)
    A = [h[0] for h in plan] + wd_tail
    B = [h[1] for h in plan]
    end = {p[2]: i + 1 for i, h in enumerate(plan) for p in h if p is not None}
    NA = len(A)
    assert NA >= NHOP + _SKEW and _LEAD >= _SKEW

    ptr = [0]

    def emit(lo, hi):
        for i in range(lo, hi):
            start(A[i], 1)
            if 0 <= i - _SKEW < NHOP and B[i - _SKEW] is not None:
                start(B[i - _SKEW], 0)

    def issue_for(e):
        hi = min(e + _LEAD, NA)
        if hi > ptr[0]:
            emit(ptr[0], hi)
            ptr[0] = hi

    def wait_all(buf, sem):
        pltpu.make_async_copy(buf, buf, sems.at[sem]).wait()

    cp_c = pltpu.make_async_copy(c_hbm, c_v, sems.at[S_C])
    cp_x = pltpu.make_async_copy(x_hbm, x_v, sems.at[S_X])
    emit(0, 1)
    ptr[0] = 1
    cp_c.start()
    cp_x.start()
    issue_for(end[S_MOD])

    row = lax.broadcasted_iota(jnp.int32, (128, G), 0)
    col = lax.broadcasted_iota(jnp.int32, (128, G), 1)
    expand = jnp.where(col // H == row, 1.0, 0.0).astype(_BF16)
    diag = (col % H) == (row % H)

    def expand_lhs(a):
        stacked = jnp.concatenate(
            [a[:, 128 * j:128 * (j + 1)] for j in range(NJ)], axis=0)
        return jnp.where(diag, _dot(stacked, expand), 0.0).astype(_BF16)

    def contract_major(big, w_v):
        out = None
        for j in range(NJ):
            t = _dot(big[H * j:H * (j + 1), :], w_v[G * j:G * (j + 1), :])
            out = t if out is None else t + out
        return out

    cp_c.wait()
    cp_x.wait()
    wait_all(wmod_v, S_MOD)
    c = c_v[...].astype(_F32)
    sc = (c * jax.nn.sigmoid(c)).astype(_BF16)
    mod = _dot(sc, _unflat(wmod_v[...], 6 * M))
    sa, ca, ga, sb, cb, gb = (mod[:, M * i:M * (i + 1)] for i in range(6))
    x = x_v[...].astype(_F32)
    h1 = (_layernorm(x) * (1.0 + ca) + sa).astype(_BF16)
    big_q = expand_lhs(jnp.broadcast_to(h1, (H, M)))

    issue_for(end[S_WQ])
    wait_all(wq_v, S_WQ)
    q = contract_major(big_q, wq_v).astype(_BF16)
    issue_for(e_pre + _X1)
    wait_all(wuk_v, S_WUK)
    ys = [_dot_nt(q, wuk_v[G * j:G * (j + 1), :]) for j in range(NJ)]
    ym = jnp.where(diag, jnp.concatenate(ys, axis=0) * (D ** -0.5), 0.0).astype(_BF16)
    qs = _dot_nt(ym, expand)
    qa = jnp.concatenate(
        [qs[H * j:H * (j + 1), :] for j in range(NJ)], axis=1).astype(_BF16)

    issue_for(e_edge + _LEAD_KV - _LEAD)
    wait_all(ckv_v.at[:, pl.ds(0, _HEAD_A)], S_KVH)
    wait_all(ckv_v.at[:, pl.ds(RKV - TAIL, TAIL)], S_KVT)
    p0 = ptr[0]
    assert p0 == e_edge + _LEAD_KV and _LEAD_KV >= _SKEW
    n_dyn = (e_kv - p0) // HPT

    def kv_step(t, carry):
        @pl.when(t < n_dyn)
        def _():
            lo = (_LEAD_KV - _SKEW) // HPS
            hi = (_LEAD_KV + HPT - 1) // HPS + 1
            hops = to_hops([kv_unit(k, g, t) for k in range(lo, hi) for g in range(_KVG)])
            for j in range(_LEAD_KV - HPS * lo, _LEAD_KV - HPS * lo + HPT):
                start(hops[j][0], 1)
                start(hops[j - _SKEW][1], 0)

        for tt in range(n_dyn, NT):
            @pl.when(t == tt)
            def _():
                emit(p0 + HPT * tt, p0 + HPT * (tt + 1))

        @pl.when(t < NT - 1)
        def _():
            wait_all(ckv_v.at[:, pl.ds(pl.multiple_of(t * FPT + _HEAD_A, 8), FPT)], S_KV + t)

        @pl.when(t == NT - 1)
        def _():
            wait_all(ckv_v.at[:, pl.ds((NT - 1) * FPT + _HEAD_A, FPT - _UNIT)], S_KV + NT - 1)

        m, l, acc = carry
        kv = _unflat(ckv_v[:, pl.ds(pl.multiple_of(t * FPT, FPT), FPT)], DC)
        s = _dot_nt(qa, kv)
        m_new = jnp.maximum(m, jnp.max(s, axis=1, keepdims=True))
        alpha = jnp.exp(m - m_new)
        p = jnp.exp(s - m_new)
        l = l * alpha + jnp.sum(p, axis=1, keepdims=True)
        acc = acc * alpha + _dot(p.astype(_BF16), kv)
        return m_new, l, acc

    init = (jnp.full((H, 1), -jnp.inf, _F32), jnp.zeros((H, 1), _F32),
            jnp.zeros((H, DC), _F32))
    _, l, acc = lax.fori_loop(0, NT, kv_step, init)
    ptr[0] = p0 + HPT * NT
    issue_for(ptr[0] - _LEAD + _X2)
    cc = (acc / l).astype(_BF16)
    big_c = expand_lhs(cc)

    issue_for(end[S_WUV])
    wait_all(wuv_v, S_WUV)
    ctx = contract_major(big_c, wuv_v)

    r32 = lax.broadcasted_iota(jnp.int32, (H, H * D), 0)
    c32 = lax.broadcasted_iota(jnp.int32, (H, H * D), 1)
    lo = jnp.where(c32 // D == r32, jnp.concatenate([ctx] * H, axis=1), 0.0).astype(_BF16)
    issue_for(max(end[S_WO], end[S_WUV] + _X3))
    wait_all(wo_v, S_WO)
    attn = jnp.sum(_dot(lo, _unflat(wo_v[...], M)), axis=0, keepdims=True)
    x2 = x + ga * attn

    h2 = (_layernorm(x2) * (1.0 + cb) + sb).astype(_BF16)
    issue_for(NA)
    wait_all(wg_v, S_WG)
    wait_all(wu_v, S_WU)

    def wait_group(i):
        for _, lo, hi in wd_groups[i]:
            wait_all(wd_v.at[pl.ds(lo, hi - lo)], S_WD0 + i)

    if _WPOS:
        wait_group(0)
    wg, wu = _unflat(wg_v[...], DF), _unflat(wu_v[...], DF)
    hcol = {}
    for blks in ((2, 3), (6, 7), (10, 11), (0, 4), (8, 12), (1, 5), (9, 13)):
        gu2 = _dot(h2, jnp.concatenate(
            [w[:, 128 * b:128 * (b + 1)] for w in (wg, wu) for b in blks], axis=1))
        hf = (jax.nn.gelu(gu2[:, :256], approximate=True) * gu2[:, 256:]).astype(_BF16).astype(_F32)
        for i, b in enumerate(blks):
            hcol[b] = jnp.broadcast_to(hf[:, 128 * i:128 * (i + 1)], (128, 128)).T
    hcol = jnp.concatenate([hcol[b] for b in range(DF // 128)], axis=0)

    done = [max(512 * g - 224, 0) for g in range(4)]
    stop = done[1:] + [DF]
    tiles = lambda v: jnp.stack([v[:, 128 * i:128 * (i + 1)] for i in range(CT)])
    acc8 = None
    for i, grp in enumerate(wd_groups):
        last = i >= _NWD - 2
        if i == _NWD - 2 and _FIN:
            rg = done[3]
            sub0 = lax.broadcasted_iota(jnp.int32, (CT, 8, 128), 1) == 0
            acc8 = acc8 * tiles(gb) + jnp.where(sub0, tiles(x2), 0.0)
            hg = hcol[done[3]:DF].reshape(-1, 1, 8, 128) * tiles(gb)
        if i or not _WPOS:
            wait_group(i)
        for g, _, hi in grp:
            r0 = done[g]
            r1 = stop[g] if hi == wd_span(g, 0, _BLK)[1] else hi // (8 * CT) * 8
            done[g] = r1
            w = wd_v[CT * r0:CT * r1, :].astype(_F32).reshape(-1, CT, 8, 128)
            t8 = jnp.sum(w * (hg[(r0 - rg) // 8:(r1 - rg) // 8] if last and _FIN else hcol[r0:r1].reshape(-1, 1, 8, 128)), axis=0)
            acc8 = t8 if acc8 is None else t8 + acc8
    ffn = jnp.sum(acc8, axis=1, keepdims=True)
    if _FIN == 2:
        for i in range(CT):
            o_ref[:, 128 * i:128 * (i + 1)] = ffn[i].astype(o_ref.dtype)
    else:
        y = jnp.concatenate([ffn[i] for i in range(CT)], axis=1)
        if not _FIN:
            y = x2 + gb * y
        o_ref[...] = y.astype(o_ref.dtype)


def _flat(a, regions=None):
    a = a.reshape(-1, a.shape[-1])
    r, c = a.shape
    a = a.reshape(r // 8, 8, c // 128, 128).transpose(0, 2, 1, 3)
    return a.reshape(-1, 128) if regions is None else a.reshape(regions, -1, 128)


@jax.jit
def pallas_adaLN_cond__compressed_kv_cla__glu_gated_geglu__decode_kernel(
    A_x, A_c_kv, A_w_q, A_w_uk, A_w_uv, A_w_o, B_x, B_w_gate, B_w_up, B_w_down, c, w_mod,
):
    B, SQ, M = A_x.shape
    _, SK, DC = A_c_kv.shape
    _, H, D = A_w_q.shape
    DF = B_w_gate.shape[1]
    assert (B, SQ, M, DC, H, D) == (1, 1, 512, 512, 32, 128) and SK % _KV_TILE == 0

    x2d = A_x.reshape(1, M)
    ckv = _flat(A_c_kv, _KVG)
    wq = A_w_q.reshape(M * H, D)
    wuk = A_w_uk.reshape(DC * H, D)
    wuv = A_w_uv.reshape(DC * H, D)
    wo = _flat(A_w_o)
    wg = _flat(B_w_gate)
    wu = _flat(B_w_up)
    wd = _flat(B_w_down)
    wmod = _flat(w_mod)
    NT = SK // _KV_TILE

    operands = (x2d, ckv, wq, wuk, wuv, wo, wg, wu, wd, c, wmod)
    vm = lambda a: pltpu.VMEM(a.shape, a.dtype)
    out = pl.pallas_call(
        functools.partial(_kernel, H=H, D=D, M=M, DC=DC, SK=SK, DF=DF),
        in_specs=[pl.BlockSpec(memory_space=pl.ANY)] * len(operands),
        out_specs=pl.BlockSpec(memory_space=pltpu.VMEM),
        out_shape=jax.ShapeDtypeStruct((1, M), A_x.dtype),
        scratch_shapes=[
            vm(x2d), vm(c), vm(wmod), vm(wq), vm(wuk), vm(ckv), vm(wuv), vm(wo),
            vm(wg), vm(wu), vm(wd),
            pltpu.SemaphoreType.DMA((S_KV + NT,)),
        ],
        compiler_params=pltpu.CompilerParams(
            vmem_limit_bytes=96 * 1024 * 1024,
            disable_semaphore_checks=True,
        ),
    )(*operands)
    return out.reshape(B, SQ, M)
```

```python
import functools

import jax
import jax.numpy as jnp
from jax import lax
import jax.experimental.pallas as pl
import jax.experimental.pallas.tpu as pltpu

_F32 = jnp.float32
_BF16 = jnp.bfloat16

_KV_TILE = 2048
_KVG = 8
_SKEW = 26
_LEAD = 48
_LEAD_KV = 72
_UNIT = 256
_BLK = 8
_HEAD_A = 112
_HEAD_F = 120
_HEAD_M = 128

(S_MOD, S_C, S_X, S_WQ, S_WUK, S_WUV, S_WO, S_WG, S_WU, S_KVH, S_KVT, S_WD0) = range(12)
_NWD = 10
S_KV = S_WD0 + _NWD


def _layernorm(x, eps=1e-05):
    m = jnp.mean(x, axis=-1, keepdims=True)
    xc = x - m
    v = jnp.mean(xc * xc, axis=-1, keepdims=True)
    return xc / jnp.sqrt(v + eps)


def _dot(a, b):
    return jnp.dot(a, b, preferred_element_type=_F32)


def _dot_nt(a, b):
    return lax.dot_general(a, b, (((1,), (1,)), ((), ())),
                           preferred_element_type=_F32)


def _unflat(v, cols):
    ct = cols // 128
    v = v.reshape(-1, ct, 8, 128)
    rows = v.shape[0] * 8
    return jnp.concatenate([v[:, i].reshape(rows, 128) for i in range(ct)], axis=1)


def _merge(*streams):
    keyed = []
    for si, s in enumerate(streams):
        for i, h in enumerate(s):
            keyed.append(((i + 0.5) / len(s), si, h))
    keyed.sort(key=lambda t: (t[0], t[1]))
    return [h for _, _, h in keyed]


def _round_robin(seq, regions):
    cut = [round(len(seq) * g / regions) for g in range(regions + 1)]
    runs = [seq[cut[g]:cut[g + 1]] for g in range(regions)]
    return [r[p] for p in range(max(map(len, runs))) for r in runs if p < len(r)]


def _kernel(x_hbm, ckv_hbm, wq_hbm, wuk_hbm, wuv_hbm, wo_hbm, wg_hbm, wu_hbm,
            wd_hbm, c_hbm, wmod_hbm, o_ref,
            x_v, c_v, wmod_v, wq_v, wuk_v, ckv_v, wuv_v, wo_v, wg_v, wu_v, wd_v,
            sems, *, H, D, M, DC, SK, DF):
    NT = SK // _KV_TILE
    RKV = ckv_hbm.shape[1]
    FPT = RKV // NT
    UPT = FPT // _UNIT
    HPS = 3 * _KVG // 4
    HPT = HPS * UPT
    G = 128 * H
    NJ = DC // 128

    def start(piece, priority):
        src, dst, sem, g, r0, rows = piece[:6]
        if not isinstance(r0, int):
            r0 = pl.multiple_of(r0, 8)
        idx = (pl.ds(r0, rows),) if g is None else (g, pl.ds(r0, rows))
        pltpu.make_async_copy(src.at[idx], dst.at[idx], sems.at[sem]).start(priority=priority)

    def units(src, dst, sem, head):
        n = src.shape[0]
        return [(src, dst, sem, None, 0, head, _UNIT - head)] + [
            (src, dst, sem, None, r, min(_UNIT, n - r), 0) for r in range(head, n, _UNIT)]

    def cut(piece, at):
        src, dst, sem, g, r0, rows, rel = piece
        pts = [rel] + [p for p in at if rel < p < rel + rows] + [rel + rows]
        return [(src, dst, sem, g, r0 + (lo - rel), hi - lo) for lo, hi in zip(pts, pts[1:])]

    def to_hops(seq):
        out = []
        for i in range(0, len(seq), 4):
            grp = seq[i:i + 4]
            if len(grp) < 4:
                out += [(u, None) for u in grp]
            else:
                b = cut(grp[0], (_UNIT // 4, 3 * _UNIT // 4))
                out += list(zip(grp[1:], b + [None] * (3 - len(b))))
        return out

    def kv_unit(k, g, t=0):
        return (ckv_hbm, ckv_v, S_KV + t + k // UPT, g, t * FPT + (_HEAD_A + _UNIT * k), _UNIT, 0)

    NK = RKV // _UNIT - 1
    TAIL = _UNIT - _HEAD_A
    h_edge = [((ckv_hbm, ckv_v, S_KVH, g, 0, _HEAD_A), (ckv_hbm, ckv_v, S_KVT, g, RKV - TAIL, TAIL))
              for g in range(_KVG)]
    h_kv = to_hops([kv_unit(k, g) for k in range(NK) for g in range(_KVG)])

    qk = _round_robin(units(wuk_hbm, wuk_v, S_WUK, _HEAD_A) + units(wq_hbm, wq_v, S_WQ, _HEAD_A), 8)
    h_pre = to_hops(_merge(_round_robin(units(wmod_hbm, wmod_v, S_MOD, _HEAD_M), 4), qk[:48]) + qk[48:])
    uvo = _round_robin(units(wo_hbm, wo_v, S_WO, _HEAD_A) + units(wuv_hbm, wuv_v, S_WUV, _HEAD_A), 8)
    gul = units(wu_hbm, wu_v, S_WU, _HEAD_F) + units(wg_hbm, wg_v, S_WG, _HEAD_F)
    cuts = [1, 9, 17, 25, 34, 42, 50, 58]
    assert len(gul) == cuts[-1]
    gu = gul[:1] + [gul[lo + p] for p in range(_BLK + 1)
                    for lo, hi in zip(cuts, cuts[1:]) if lo + p < hi]

    FD = wd_hbm.shape[0]
    CT = M // 128

    def wd_span(g, j0, j1):
        o = _BLK * _UNIT * g + _HEAD_F - 4 * _UNIT
        return max(o + _UNIT * j0, 0), min(o + _UNIT * j1, FD)

    wd_groups = ([[(g,) + wd_span(g, 0, 3) for g in (1, 2, 3)]]
                 + [[(g,) + wd_span(g, j, j + 1) for g in range(4)] for j in range(3, 7)]
                 + [[(g,) + wd_span(g, 7, 8)] for g in range(3)]
                 + [[(3, wd_span(3, 7, 8)[0], FD - 40)], [(3, FD - 40, FD)]])
    assert len(wd_groups) == _NWD and wd_span(3, 0, _BLK)[1] == FD
    wd_seq = [(wd_hbm, wd_v, S_WD0 + max(j - 2, 0), None, lo, hi - lo, _UNIT - (hi - lo))
              for j in range(7) for lo, hi in (wd_span(g, j, j + 1) for g in range(4)) if hi > lo]
    wd_tail = [p for i in range(5, _NWD) for _, lo, hi in wd_groups[i]
               for p in cut((wd_hbm, wd_v, S_WD0 + i, None, lo, hi - lo, 0), range(32, hi - lo - 16, 32))]
    mix = "gg" + "ggggdggg" * 7 + "dgggdgggdg"
    assert mix.count("g") == len(gu)
    its = {"g": iter(gu), "d": iter(wd_seq)}
    h_post = to_hops(uvo + [next(its[ch]) for ch in mix] + list(its["d"]))

    plan = h_pre + h_edge + h_kv + h_post
    e_pre = len(h_pre)
    e_edge = e_pre + len(h_edge)
    e_kv = e_edge + len(h_kv)
    NHOP = len(plan)
    A = [h[0] for h in plan] + wd_tail
    B = [h[1] for h in plan]
    end = {p[2]: i + 1 for i, h in enumerate(plan) for p in h if p is not None}
    NA = len(A)
    assert NA >= NHOP + _SKEW and _LEAD >= _SKEW

    ptr = [0]

    def emit(lo, hi):
        for i in range(lo, hi):
            start(A[i], 1)
            if 0 <= i - _SKEW < NHOP and B[i - _SKEW] is not None:
                start(B[i - _SKEW], 0)

    def issue_for(e):
        hi = min(e + _LEAD, NA)
        if hi > ptr[0]:
            emit(ptr[0], hi)
            ptr[0] = hi

    def wait_all(buf, sem):
        pltpu.make_async_copy(buf, buf, sems.at[sem]).wait()

    cp_c = pltpu.make_async_copy(c_hbm, c_v, sems.at[S_C])
    cp_x = pltpu.make_async_copy(x_hbm, x_v, sems.at[S_X])
    emit(0, 1)
    ptr[0] = 1
    cp_c.start()
    cp_x.start()
    issue_for(end[S_MOD])

    row = lax.broadcasted_iota(jnp.int32, (128, G), 0)
    col = lax.broadcasted_iota(jnp.int32, (128, G), 1)
    expand = jnp.where(col // H == row, 1.0, 0.0).astype(_BF16)
    diag = (col % H) == (row % H)

    def expand_lhs(a):
        stacked = jnp.concatenate(
            [a[:, 128 * j:128 * (j + 1)] for j in range(NJ)], axis=0)
        return jnp.where(diag, _dot(stacked, expand), 0.0).astype(_BF16)

    def contract_major(big, w_v):
        out = None
        for j in range(NJ):
            t = _dot(big[H * j:H * (j + 1), :], w_v[G * j:G * (j + 1), :])
            out = t if out is None else t + out
        return out

    cp_c.wait()
    cp_x.wait()
    wait_all(wmod_v, S_MOD)
    c = c_v[...].astype(_F32)
    sc = (c * jax.nn.sigmoid(c)).astype(_BF16)
    mod = _dot(sc, _unflat(wmod_v[...], 6 * M))
    sa, ca, ga, sb, cb, gb = (mod[:, M * i:M * (i + 1)] for i in range(6))
    x = x_v[...].astype(_F32)
    h1 = (_layernorm(x) * (1.0 + ca) + sa).astype(_BF16)
    big_q = expand_lhs(jnp.broadcast_to(h1, (H, M)))

    issue_for(end[S_WQ])
    wait_all(wq_v, S_WQ)
    q = contract_major(big_q, wq_v).astype(_BF16)
    issue_for(e_pre + 12)
    wait_all(wuk_v, S_WUK)
    ys = [_dot_nt(q, wuk_v[G * j:G * (j + 1), :]) for j in range(NJ)]
    ym = jnp.where(diag, jnp.concatenate(ys, axis=0) * (D ** -0.5), 0.0).astype(_BF16)
    qs = _dot_nt(ym, expand)
    qa = jnp.concatenate(
        [qs[H * j:H * (j + 1), :] for j in range(NJ)], axis=1).astype(_BF16)

    issue_for(e_edge + _LEAD_KV - _LEAD)
    wait_all(ckv_v.at[:, pl.ds(0, _HEAD_A)], S_KVH)
    wait_all(ckv_v.at[:, pl.ds(RKV - TAIL, TAIL)], S_KVT)
    p0 = ptr[0]
    assert p0 == e_edge + _LEAD_KV and _LEAD_KV >= _SKEW
    n_dyn = (e_kv - p0) // HPT

    def kv_step(t, carry):
        @pl.when(t < n_dyn)
        def _():
            lo = (_LEAD_KV - _SKEW) // HPS
            hi = (_LEAD_KV + HPT - 1) // HPS + 1
            hops = to_hops([kv_unit(k, g, t) for k in range(lo, hi) for g in range(_KVG)])
            for j in range(_LEAD_KV - HPS * lo, _LEAD_KV - HPS * lo + HPT):
                start(hops[j][0], 1)
                start(hops[j - _SKEW][1], 0)

        for tt in range(n_dyn, NT):
            @pl.when(t == tt)
            def _():
                emit(p0 + HPT * tt, p0 + HPT * (tt + 1))

        @pl.when(t < NT - 1)
        def _():
            wait_all(ckv_v.at[:, pl.ds(pl.multiple_of(t * FPT + _HEAD_A, 8), FPT)], S_KV + t)

        @pl.when(t == NT - 1)
        def _():
            wait_all(ckv_v.at[:, pl.ds((NT - 1) * FPT + _HEAD_A, FPT - _UNIT)], S_KV + NT - 1)

        m, l, acc = carry
        kv = _unflat(ckv_v[:, pl.ds(pl.multiple_of(t * FPT, FPT), FPT)], DC)
        s = _dot_nt(qa, kv)
        m_new = jnp.maximum(m, jnp.max(s, axis=1, keepdims=True))
        alpha = jnp.exp(m - m_new)
        p = jnp.exp(s - m_new)
        l = l * alpha + jnp.sum(p, axis=1, keepdims=True)
        acc = acc * alpha + _dot(p.astype(_BF16), kv)
        return m_new, l, acc

    init = (jnp.full((H, 1), -jnp.inf, _F32), jnp.zeros((H, 1), _F32),
            jnp.zeros((H, DC), _F32))
    _, l, acc = lax.fori_loop(0, NT, kv_step, init)
    ptr[0] = p0 + HPT * NT
    issue_for(ptr[0] - _LEAD + 14)
    cc = (acc / l).astype(_BF16)
    big_c = expand_lhs(cc)

    issue_for(end[S_WUV])
    wait_all(wuv_v, S_WUV)
    ctx = contract_major(big_c, wuv_v)

    r32 = lax.broadcasted_iota(jnp.int32, (H, H * D), 0)
    c32 = lax.broadcasted_iota(jnp.int32, (H, H * D), 1)
    lo = jnp.where(c32 // D == r32, jnp.concatenate([ctx] * H, axis=1), 0.0).astype(_BF16)
    issue_for(max(end[S_WO], end[S_WUV] + 8))
    wait_all(wo_v, S_WO)
    attn = jnp.sum(_dot(lo, _unflat(wo_v[...], M)), axis=0, keepdims=True)
    x2 = x + ga * attn

    h2 = (_layernorm(x2) * (1.0 + cb) + sb).astype(_BF16)
    issue_for(NA)
    wait_all(wg_v, S_WG)
    wait_all(wu_v, S_WU)

    def wait_group(i):
        for _, lo, hi in wd_groups[i]:
            wait_all(wd_v.at[pl.ds(lo, hi - lo)], S_WD0 + i)

    wait_group(0)
    wg, wu = _unflat(wg_v[...], DF), _unflat(wu_v[...], DF)
    hcol = {}
    for blks in ((2, 3), (6, 7), (10, 11), (0, 4), (8, 12), (1, 5), (9, 13)):
        gu2 = _dot(h2, jnp.concatenate(
            [w[:, 128 * b:128 * (b + 1)] for w in (wg, wu) for b in blks], axis=1))
        hf = (jax.nn.gelu(gu2[:, :256], approximate=True) * gu2[:, 256:]).astype(_BF16).astype(_F32)
        for i, b in enumerate(blks):
            hcol[b] = jnp.broadcast_to(hf[:, 128 * i:128 * (i + 1)], (128, 128)).T
    hcol = jnp.concatenate([hcol[b] for b in range(DF // 128)], axis=0)

    done = [max(512 * g - 224, 0) for g in range(4)]
    stop = done[1:] + [DF]
    tiles = lambda v: jnp.stack([v[:, 128 * i:128 * (i + 1)] for i in range(CT)])
    coef = hcol.reshape(-1, 1, 8, 128)
    acc8 = None
    for i, grp in enumerate(wd_groups):
        if i == _NWD - 2:
            sub0 = lax.broadcasted_iota(jnp.int32, (CT, 8, 128), 1) == 0
            acc8 = acc8 * tiles(gb) + jnp.where(sub0, tiles(x2), 0.0)
            rest = done[3] // 8
            coef = coef[rest:] * tiles(gb)
        elif i < _NWD - 2:
            rest = 0
        if i:
            wait_group(i)
        for g, _, hi in grp:
            r0 = done[g]
            r1 = stop[g] if hi == wd_span(g, 0, _BLK)[1] else hi // (8 * CT) * 8
            done[g] = r1
            w = wd_v[CT * r0:CT * r1, :].astype(_F32).reshape(-1, CT, 8, 128)
            t8 = jnp.sum(w * coef[r0 // 8 - rest:r1 // 8 - rest], axis=0)
            acc8 = t8 if acc8 is None else t8 + acc8
    assert done == stop
    y = jnp.sum(acc8, axis=1, keepdims=True)
    for i in range(CT):
        o_ref[:, 128 * i:128 * (i + 1)] = y[i].astype(o_ref.dtype)


def _flat(a, regions=None):
    a = a.reshape(-1, a.shape[-1])
    r, c = a.shape
    a = a.reshape(r // 8, 8, c // 128, 128).transpose(0, 2, 1, 3)
    return a.reshape(-1, 128) if regions is None else a.reshape(regions, -1, 128)


@jax.jit
def pallas_adaLN_cond__compressed_kv_cla__glu_gated_geglu__decode_kernel(
    A_x, A_c_kv, A_w_q, A_w_uk, A_w_uv, A_w_o, B_x, B_w_gate, B_w_up, B_w_down, c, w_mod,
):
    B, SQ, M = A_x.shape
    _, SK, DC = A_c_kv.shape
    _, H, D = A_w_q.shape
    DF = B_w_gate.shape[1]
    assert (B, SQ, M, DC, H, D, SK, DF) == (1, 1, 512, 512, 32, 128, 32768, 1792)

    x2d = A_x.reshape(1, M)
    ckv = _flat(A_c_kv, _KVG)
    wq = A_w_q.reshape(M * H, D)
    wuk = A_w_uk.reshape(DC * H, D)
    wuv = A_w_uv.reshape(DC * H, D)
    wo = _flat(A_w_o)
    wg = _flat(B_w_gate)
    wu = _flat(B_w_up)
    wd = _flat(B_w_down)
    wmod = _flat(w_mod)
    NT = SK // _KV_TILE

    operands = (x2d, ckv, wq, wuk, wuv, wo, wg, wu, wd, c, wmod)
    vm = lambda a: pltpu.VMEM(a.shape, a.dtype)
    out = pl.pallas_call(
        functools.partial(_kernel, H=H, D=D, M=M, DC=DC, SK=SK, DF=DF),
        in_specs=[pl.BlockSpec(memory_space=pl.ANY)] * len(operands),
        out_specs=pl.BlockSpec(memory_space=pltpu.VMEM),
        out_shape=jax.ShapeDtypeStruct((1, M), A_x.dtype),
        scratch_shapes=[
            vm(x2d), vm(c), vm(wmod), vm(wq), vm(wuk), vm(ckv), vm(wuv), vm(wo),
            vm(wg), vm(wu), vm(wd),
            pltpu.SemaphoreType.DMA((S_KV + NT,)),
        ],
        compiler_params=pltpu.CompilerParams(
            vmem_limit_bytes=96 * 1024 * 1024,
            disable_semaphore_checks=True,
        ),
    )(*operands)
    return out.reshape(B, SQ, M)
```

```python
import functools

import jax
import jax.numpy as jnp
from jax import lax
import jax.experimental.pallas as pl
import jax.experimental.pallas.tpu as pltpu

_F32 = jnp.float32
_BF16 = jnp.bfloat16

_KV_TILE = 2048
_KVG = 8
_SKEW = 25
_LEAD = 52
_LEAD_KV = 80
_UNIT = 256
_BLK = 8
_HEAD_A = 112
_HEAD_F = 120
_HEAD_M = 128

(S_MOD, S_C, S_X, S_WQ, S_WUK, S_WUV, S_WO, S_WG, S_WU, S_KVH, S_KVT, S_WD0) = range(12)
_NWD = 10
S_KV = S_WD0 + _NWD


def _layernorm(x, eps=1e-05):
    m = jnp.mean(x, axis=-1, keepdims=True)
    xc = x - m
    v = jnp.mean(xc * xc, axis=-1, keepdims=True)
    return xc / jnp.sqrt(v + eps)


def _dot(a, b):
    return jnp.dot(a, b, preferred_element_type=_F32)


def _dot_nt(a, b):
    return lax.dot_general(a, b, (((1,), (1,)), ((), ())),
                           preferred_element_type=_F32)


def _unflat(v, cols):
    ct = cols // 128
    v = v.reshape(-1, ct, 8, 128)
    rows = v.shape[0] * 8
    return jnp.concatenate([v[:, i].reshape(rows, 128) for i in range(ct)], axis=1)


def _merge(*streams):
    keyed = []
    for si, s in enumerate(streams):
        for i, h in enumerate(s):
            keyed.append(((i + 0.5) / len(s), si, h))
    keyed.sort(key=lambda t: (t[0], t[1]))
    return [h for _, _, h in keyed]


def _round_robin(seq, regions):
    cut = [round(len(seq) * g / regions) for g in range(regions + 1)]
    runs = [seq[cut[g]:cut[g + 1]] for g in range(regions)]
    return [r[p] for p in range(max(map(len, runs))) for r in runs if p < len(r)]


def _kernel(x_hbm, ckv_hbm, wq_hbm, wuk_hbm, wuv_hbm, wo_hbm, wg_hbm, wu_hbm,
            wd_hbm, c_hbm, wmod_hbm, o_ref,
            x_v, c_v, wmod_v, wq_v, wuk_v, ckv_v, wuv_v, wo_v, wg_v, wu_v, wd_v,
            sems, *, H, D, M, DC, SK, DF):
    NT = SK // _KV_TILE
    RKV = ckv_hbm.shape[1]
    FPT = RKV // NT
    UPT = FPT // _UNIT
    HPT = _KVG * UPT
    G = 128 * H
    NJ = DC // 128

    def start(piece, priority):
        src, dst, sem, g, r0, rows = piece[:6]
        if not isinstance(r0, int):
            r0 = pl.multiple_of(r0, 8)
        idx = (pl.ds(r0, rows),) if g is None else (g, pl.ds(r0, rows))
        pltpu.make_async_copy(src.at[idx], dst.at[idx], sems.at[sem]).start(priority=priority)

    def units(src, dst, sem, head):
        n = src.shape[0]
        return [(src, dst, sem, None, 0, head, _UNIT - head)] + [
            (src, dst, sem, None, r, min(_UNIT, n - r), 0) for r in range(head, n, _UNIT)]

    def cut(piece, at):
        src, dst, sem, g, r0, rows, rel = piece
        pts = [rel] + [p for p in at if rel < p < rel + rows] + [rel + rows]
        return [(src, dst, sem, g, r0 + (lo - rel), hi - lo) for lo, hi in zip(pts, pts[1:])]

    def to_hops(seq):
        return [tuple(cut(u, (3 * _UNIT // 4 if u[6] else _UNIT // 4,))[::-1]) for u in seq]

    def pair_hops(lo, hi):
        return to_hops(lo[:-1]) + [(lo[-1], hi[0])] + to_hops(hi[1:])

    def kv_unit(k, g, t=0):
        return (ckv_hbm, ckv_v, S_KV + t + k // UPT, g, t * FPT + (_HEAD_A + _UNIT * k), _UNIT, 0)

    NK = RKV // _UNIT - 1
    TAIL = _UNIT - _HEAD_A
    heads = [(ckv_hbm, ckv_v, S_KVH, g, 0, _HEAD_A, TAIL) for g in range(_KVG)]
    tails = [(ckv_hbm, ckv_v, S_KVT, g, RKV - TAIL, TAIL, 0) for g in range(_KVG)]
    h_edge = to_hops(heads[:1]) + list(zip(tails, heads[1:])) + to_hops(tails[-1:])
    h_kv = to_hops([kv_unit(k, g) for k in range(NK) for g in range(_KVG)])

    qk = _round_robin(pair_hops(units(wuk_hbm, wuk_v, S_WUK, _HEAD_A),
                                units(wq_hbm, wq_v, S_WQ, _HEAD_A)), 8)
    h_pre = _merge(_round_robin(to_hops(units(wmod_hbm, wmod_v, S_MOD, _HEAD_M)), 4), qk[:48]) + qk[48:]
    uvo = _round_robin(pair_hops(units(wo_hbm, wo_v, S_WO, _HEAD_A),
                                 units(wuv_hbm, wuv_v, S_WUV, _HEAD_A)), 8)
    gu = pair_hops(units(wu_hbm, wu_v, S_WU, _HEAD_F), units(wg_hbm, wg_v, S_WG, _HEAD_F))
    gu = gu[:1] + _round_robin(gu[1:], len(gu) // _BLK)

    FD = wd_hbm.shape[0]
    CT = M // 128

    def wd_span(g, j0, j1):
        o = _BLK * _UNIT * g + _HEAD_F - 4 * _UNIT
        return max(o + _UNIT * j0, 0), min(o + _UNIT * j1, FD)

    wd_groups = ([[(g,) + wd_span(g, 0, 3) for g in (1, 2, 3)]]
                 + [[(g,) + wd_span(g, j, j + 1) for g in range(4)] for j in range(3, 7)]
                 + [[(g,) + wd_span(g, 7, 8)] for g in range(3)]
                 + [[(3, wd_span(3, 7, 8)[0], FD - 40)], [(3, FD - 40, FD)]])
    assert len(wd_groups) == _NWD and wd_span(3, 0, _BLK)[1] == FD
    wd_piece = lambda i, lo, hi: (wd_hbm, wd_v, S_WD0 + i, None, lo, hi - lo, _UNIT - hi if lo == 0 else 0)
    h_wd = to_hops([wd_piece(0, *wd_span(g, j, j + 1)) for j in range(3) for g in (1, 2, 3)]
                   + [wd_piece(i, lo, hi) for i in range(1, 7) for _, lo, hi in wd_groups[i]])
    wd_tail = [p for i in range(7, _NWD) for _, lo, hi in wd_groups[i]
               for p in cut(wd_piece(i, lo, hi), range(16, hi - lo, 16))]
    h_post = uvo + _merge(gu, h_wd[:6]) + h_wd[6:]

    plan = h_pre + h_edge + h_kv + h_post
    e_pre = len(h_pre)
    e_edge = e_pre + len(h_edge)
    e_kv = e_edge + len(h_kv)
    NHOP = len(plan)
    A = [h[0] for h in plan] + wd_tail
    B = [h[1] for h in plan]
    end = {p[2]: i + 1 for i, h in enumerate(plan) for p in h}
    NA = len(A)
    assert NA >= NHOP + _SKEW and _LEAD >= _SKEW

    ptr = [0]

    def emit(lo, hi):
        for i in range(lo, hi):
            start(A[i], 1)
            if 0 <= i - _SKEW < NHOP:
                start(B[i - _SKEW], 0)

    def issue_for(e):
        hi = min(e + _LEAD, NA)
        if hi > ptr[0]:
            emit(ptr[0], hi)
            ptr[0] = hi

    def wait_all(buf, sem):
        pltpu.make_async_copy(buf, buf, sems.at[sem]).wait()

    cp_c = pltpu.make_async_copy(c_hbm, c_v, sems.at[S_C])
    cp_x = pltpu.make_async_copy(x_hbm, x_v, sems.at[S_X])
    emit(0, 1)
    ptr[0] = 1
    cp_c.start()
    cp_x.start()
    issue_for(end[S_MOD])

    row = lax.broadcasted_iota(jnp.int32, (128, G), 0)
    col = lax.broadcasted_iota(jnp.int32, (128, G), 1)
    expand = jnp.where(col // H == row, 1.0, 0.0).astype(_BF16)
    diag = (col % H) == (row % H)

    def expand_lhs(a):
        stacked = jnp.concatenate(
            [a[:, 128 * j:128 * (j + 1)] for j in range(NJ)], axis=0)
        return jnp.where(diag, _dot(stacked, expand), 0.0).astype(_BF16)

    def contract_major(big, w_v):
        out = None
        for j in range(NJ):
            t = _dot(big[H * j:H * (j + 1), :], w_v[G * j:G * (j + 1), :])
            out = t if out is None else t + out
        return out

    cp_c.wait()
    cp_x.wait()
    wait_all(wmod_v, S_MOD)
    c = c_v[...].astype(_F32)
    sc = (c * jax.nn.sigmoid(c)).astype(_BF16)
    mod = _dot(sc, _unflat(wmod_v[...], 6 * M))
    sa, ca, ga, sb, cb, gb = (mod[:, M * i:M * (i + 1)] for i in range(6))
    x = x_v[...].astype(_F32)
    h1 = (_layernorm(x) * (1.0 + ca) + sa).astype(_BF16)
    big_q = expand_lhs(jnp.broadcast_to(h1, (H, M)))

    issue_for(end[S_WQ])
    wait_all(wq_v, S_WQ)
    q = contract_major(big_q, wq_v).astype(_BF16)
    issue_for(e_pre + 10)
    wait_all(wuk_v, S_WUK)
    ys = [_dot_nt(q, wuk_v[G * j:G * (j + 1), :]) for j in range(NJ)]
    issue_for(e_pre + 26)
    ym = jnp.where(diag, jnp.concatenate(ys, axis=0) * (D ** -0.5), 0.0).astype(_BF16)
    qs = _dot_nt(ym, expand)
    qa = jnp.concatenate(
        [qs[H * j:H * (j + 1), :] for j in range(NJ)], axis=1).astype(_BF16)

    issue_for(e_edge + _LEAD_KV - _LEAD)
    wait_all(ckv_v.at[:, pl.ds(0, _HEAD_A)], S_KVH)
    wait_all(ckv_v.at[:, pl.ds(RKV - TAIL, TAIL)], S_KVT)
    p0 = ptr[0]
    assert p0 == e_edge + _LEAD_KV and _LEAD_KV >= _SKEW
    n_dyn = (e_kv - p0) // HPT

    def kv_step(t, carry):
        @pl.when(t < n_dyn)
        def _():
            for h in range(_LEAD_KV, _LEAD_KV + HPT):
                (a, _), (_, b) = to_hops([kv_unit(*divmod(i, _KVG), t) for i in (h, h - _SKEW)])
                start(a, 1)
                start(b, 0)

        for tt in range(n_dyn, NT):
            @pl.when(t == tt)
            def _():
                emit(p0 + HPT * tt, p0 + HPT * (tt + 1))

        @pl.when(t < NT - 1)
        def _():
            wait_all(ckv_v.at[:, pl.ds(pl.multiple_of(t * FPT + _HEAD_A, 8), FPT)], S_KV + t)

        @pl.when(t == NT - 1)
        def _():
            wait_all(ckv_v.at[:, pl.ds((NT - 1) * FPT + _HEAD_A, FPT - _UNIT)], S_KV + NT - 1)

        m, l, acc = carry
        kv = _unflat(ckv_v[:, pl.ds(pl.multiple_of(t * FPT, FPT), FPT)], DC)
        s = _dot_nt(qa, kv)
        m_new = jnp.maximum(m, jnp.max(s, axis=1, keepdims=True))
        alpha = jnp.exp(m - m_new)
        p = jnp.exp(s - m_new)
        l = l * alpha + jnp.sum(p, axis=1, keepdims=True)
        acc = acc * alpha + _dot(p.astype(_BF16), kv)
        return m_new, l, acc

    init = (jnp.full((H, 1), -jnp.inf, _F32), jnp.zeros((H, 1), _F32),
            jnp.zeros((H, DC), _F32))
    _, l, acc = lax.fori_loop(0, NT, kv_step, init)
    ptr[0] = p0 + HPT * NT
    issue_for(ptr[0] - _LEAD + 16)
    cc = (acc / l).astype(_BF16)
    big_c = expand_lhs(cc)

    issue_for(end[S_WUV])
    wait_all(wuv_v, S_WUV)
    ctx = contract_major(big_c, wuv_v)

    r32 = lax.broadcasted_iota(jnp.int32, (H, H * D), 0)
    c32 = lax.broadcasted_iota(jnp.int32, (H, H * D), 1)
    lo = jnp.where(c32 // D == r32, jnp.concatenate([ctx] * H, axis=1), 0.0).astype(_BF16)
    issue_for(max(end[S_WO], end[S_WUV] + 10))
    wait_all(wo_v, S_WO)
    attn = jnp.sum(_dot(lo, _unflat(wo_v[...], M)), axis=0, keepdims=True)
    x2 = x + ga * attn

    h2 = (_layernorm(x2) * (1.0 + cb) + sb).astype(_BF16)
    issue_for(NA)
    wait_all(wg_v, S_WG)
    wait_all(wu_v, S_WU)
    wg, wu = _unflat(wg_v[...], DF), _unflat(wu_v[...], DF)
    hcol = {}
    for blks in ((2, 3), (6, 7), (10, 11), (0, 4), (8, 12), (1, 5), (9, 13)):
        gu2 = _dot(h2, jnp.concatenate(
            [w[:, 128 * b:128 * (b + 1)] for w in (wg, wu) for b in blks], axis=1))
        hf = (jax.nn.gelu(gu2[:, :256], approximate=True) * gu2[:, 256:]).astype(_BF16).astype(_F32)
        for i, b in enumerate(blks):
            hcol[b] = jnp.broadcast_to(hf[:, 128 * i:128 * (i + 1)], (128, 128)).T
    hcol = jnp.concatenate([hcol[b] for b in range(DF // 128)], axis=0)

    done = [max(512 * g - 224, 0) for g in range(4)]
    stop = done[1:] + [DF]
    tiles = lambda v: jnp.stack([v[:, 128 * i:128 * (i + 1)] for i in range(CT)])
    coef = hcol.reshape(-1, 1, 8, 128)
    acc8 = None
    late = {}
    for i, grp in enumerate(wd_groups):
        if i == _NWD - 3:
            sub0 = lax.broadcasted_iota(jnp.int32, (CT, 8, 128), 1) == 0
            acc8 = acc8 * tiles(gb) + jnp.where(sub0, tiles(x2), 0.0)
            late = {g: (done[g] // 8, coef[done[g] // 8:stop[g] // 8] * tiles(gb))
                    for g in range(4) if done[g] < stop[g]}
        for _, lo, hi in grp:
            wait_all(wd_v.at[pl.ds(lo, hi - lo)], S_WD0 + i)
        for g, _, hi in grp:
            r0 = done[g]
            r1 = stop[g] if hi == wd_span(g, 0, _BLK)[1] else hi // (8 * CT) * 8
            done[g] = r1
            w = wd_v[CT * r0:CT * r1, :].astype(_F32).reshape(-1, CT, 8, 128)
            off, cf = late.get(g, (0, coef))
            t8 = jnp.sum(w * cf[r0 // 8 - off:r1 // 8 - off], axis=0)
            acc8 = t8 if acc8 is None else t8 + acc8
    assert done == stop
    y = jnp.sum(acc8, axis=1, keepdims=True)
    for i in range(CT):
        o_ref[:, 128 * i:128 * (i + 1)] = y[i].astype(o_ref.dtype)


def _flat(a, regions=None):
    a = a.reshape(-1, a.shape[-1])
    r, c = a.shape
    a = a.reshape(r // 8, 8, c // 128, 128).transpose(0, 2, 1, 3)
    return a.reshape(-1, 128) if regions is None else a.reshape(regions, -1, 128)


@jax.jit
def pallas_adaLN_cond__compressed_kv_cla__glu_gated_geglu__decode_kernel(
    A_x, A_c_kv, A_w_q, A_w_uk, A_w_uv, A_w_o, B_x, B_w_gate, B_w_up, B_w_down, c, w_mod,
):
    B, SQ, M = A_x.shape
    _, SK, DC = A_c_kv.shape
    _, H, D = A_w_q.shape
    DF = B_w_gate.shape[1]
    assert (B, SQ, M, DC, H, D, SK, DF) == (1, 1, 512, 512, 32, 128, 32768, 1792)

    x2d = A_x.reshape(1, M)
    ckv = _flat(A_c_kv, _KVG)
    wq = A_w_q.reshape(M * H, D)
    wuk = A_w_uk.reshape(DC * H, D)
    wuv = A_w_uv.reshape(DC * H, D)
    wo = _flat(A_w_o)
    wg = _flat(B_w_gate)
    wu = _flat(B_w_up)
    wd = _flat(B_w_down)
    wmod = _flat(w_mod)
    NT = SK // _KV_TILE

    operands = (x2d, ckv, wq, wuk, wuv, wo, wg, wu, wd, c, wmod)
    vm = lambda a: pltpu.VMEM(a.shape, a.dtype)
    out = pl.pallas_call(
        functools.partial(_kernel, H=H, D=D, M=M, DC=DC, SK=SK, DF=DF),
        in_specs=[pl.BlockSpec(memory_space=pl.ANY)] * len(operands),
        out_specs=pl.BlockSpec(memory_space=pltpu.VMEM),
        out_shape=jax.ShapeDtypeStruct((1, M), A_x.dtype),
        scratch_shapes=[
            vm(x2d), vm(c), vm(wmod), vm(wq), vm(wuk), vm(ckv), vm(wuv), vm(wo),
            vm(wg), vm(wu), vm(wd),
            pltpu.SemaphoreType.DMA((S_KV + NT,)),
        ],
        compiler_params=pltpu.CompilerParams(
            vmem_limit_bytes=96 * 1024 * 1024,
            disable_semaphore_checks=True,
        ),
    )(*operands)
    return out.reshape(B, SQ, M)
```
